```python
import jax
import jax.numpy as jnp

def _softmax(x, axis=-1):
    return jax.nn.softmax(x, axis=axis)
def _gelu(x):
    return jax.nn.gelu(x, approximate=True)
def _silu(x):
    return jax.nn.silu(x)
def _sigmoid(x):
    return jax.nn.sigmoid(x)
def _layernorm(x, axis=-1, eps=1e-5):
    m = jnp.mean(x, axis=axis, keepdims=True)
    v = jnp.var(x, axis=axis, keepdims=True)
    return (x - m) / jnp.sqrt(v + eps)
def _scatter_add(tgt, idx, src, axis=0):
    return tgt.at[idx].add(src)
def _segment_sum(src, seg, n):
    return jax.ops.segment_sum(src, seg, n)
class _Rng:
    def __init__(self, key):
        self._k = key
    def _next(self):
        self._k, sub = jax.random.split(self._k)
        return sub
    def normal(self, shape):
        return jax.random.normal(self._next(), shape, dtype=jnp.bfloat16)
    def randint(self, lo, hi, shape):
        return jax.random.randint(self._next(), shape, lo, hi, dtype=jnp.int32)
    def uniform(self, shape, lo=0.0, hi=1.0):
        return jax.random.uniform(self._next(), shape, jnp.bfloat16, lo, hi)
    def permutation(self, n):
        return jax.random.permutation(self._next(), n)


kernel_name = 'concat_heads__ssm_conv_h3__sliding_local_dilated__prompt'

def setup_inputs():
    _rng = _Rng(jax.random.key(int.from_bytes(__import__("os").urandom(4), "little")))
    _w = (lambda a: (lambda t: t.astype(jnp.bfloat16) if jnp.issubdtype(t.dtype, jnp.floating) else t)(jnp.asarray(a)))
    def _A_setup():
        B, S, D = 1, 2048, 1024
        ks = 4
        return {
            "q": _w((lambda *s: _rng.normal(s) * 0.05)(B, S, D)),
            "k": _w((lambda *s: _rng.normal(s) * 0.05)(B, S, D)),
            "v": _w((lambda *s: _rng.normal(s) * 0.05)(B, S, D)),
            "shift_k": _w((lambda *s: _rng.normal(s) * 0.05)(D, ks) * 0.5),
            "ssm_k": _w((lambda *s: _rng.normal(s) * 0.05)(D, S) * (1.0 / S ** 0.5)),
            "ssm_D": _w((lambda *s: _rng.normal(s) * 0.05)(D)),
        }
    _A_in = _A_setup()

    def _B_setup():
        B, S, D = 1, 2048, 1024
        return {
            "x": _w((lambda *s: _rng.normal(s) * 0.05)(B, S, D)),
            "wqkv": _w((lambda *s: _rng.normal(s) * 0.05)(D, 3 * D)),
            "wo": _w((lambda *s: _rng.normal(s) * 0.05)(D, D)),
        }
    _B_in = _B_setup()

    return {
        "A_q": _A_in["q"],
        "A_k": _A_in["k"],
        "A_v": _A_in["v"],
        "A_shift_k": _A_in["shift_k"],
        "A_ssm_k": _A_in["ssm_k"],
        "A_ssm_D": _A_in["ssm_D"],
        "B_x": _B_in["x"],
        "B_wqkv": _B_in["wqkv"],
        "B_wo": _B_in["wo"],
    }

def reference(A_q, A_k, A_v, A_shift_k, A_ssm_k, A_ssm_D, B_x, B_wqkv, B_wo):
    def _A_ref(q, k, v, shift_k, ssm_k, ssm_D):
        B, S, D = q.shape
        ks = shift_k.shape[-1]
        k_pad = jnp.pad(k, ((0, 0), (ks - 1, 0), (0, 0)))
        k_shift = jnp.zeros_like(k)
        for t in range(ks):
            k_shift = k_shift + k_pad[:, t:t + S, :] * shift_k[:, ks - 1 - t][None, None, :]
        kv = k_shift * v
        L = 2 * S
        kv_pad = jnp.pad(kv, ((0, 0), (0, S), (0, 0)))
        kf_pad = jnp.pad(ssm_k, ((0, 0), (0, S)))
        kv_f = (lambda x, axes=(-2,-1): jnp.fft.rfft2(x.astype(jnp.float32), axes=axes))(kv_pad[:, None, :, :], axes=(1, 2))
        kf_f = (lambda x, axes=(-2,-1): jnp.fft.rfft2(x.astype(jnp.float32), axes=axes))(kf_pad[:, None, :], axes=(1, 2))
        kf_f = (lambda x, *d: x.transpose(*d))(kf_f, 1, 2, 0)
        y_f = kv_f * kf_f[None, :, :, :]
        y = (lambda x, s, axes=(-2,-1): jnp.fft.irfft2(x, s=s, axes=axes).astype(jnp.bfloat16))(y_f, (1, L), axes=(1, 2))[:, 0, :S, :]
        y = y + kv * ssm_D[None, None, :]
        return q * y

    def _B_ref(x, wqkv, wo):
        B, S, D = x.shape
        H = 32; Dh = D // H
        W, dil = 8, 2
        qkv = (lambda x, *d: x.transpose(*d))((x @ wqkv).reshape(B, S, 3, H, Dh), 2, 0, 3, 1, 4)
        q, k, v = qkv[0], qkv[1], qkv[2]
        scale = Dh ** -0.5
        pos = jnp.arange(S)
        off = jnp.arange(W) * dil
        idx = pos[:, None] - off[None, :]
        mask = idx >= 0
        idx_c = jnp.where(mask, idx, 0).reshape(-1)
        kg = k[:, :, idx_c, :].reshape(B, H, S, W, Dh)
        vg = v[:, :, idx_c, :].reshape(B, H, S, W, Dh)
        logits = jnp.einsum("bhsd,bhswd->bhsw", q, kg) * scale
        logits = jnp.where(mask[None, None, :, :], logits, -1e9)
        attn = _softmax(logits, axis=-1)
        o = jnp.einsum("bhsw,bhswd->bhsd", attn, vg)
        return (lambda x, *d: x.transpose(*d))(o, 0, 2, 1, 3).reshape(B, S, D) @ wo

    a = _A_ref(A_q, A_k, A_v, A_shift_k, A_ssm_k, A_ssm_D)
    b = _B_ref(B_x, B_wqkv, B_wo)
    return jnp.concatenate([a, b], axis=-1)
```

```python
import functools
import math

import jax
import jax.numpy as jnp
import numpy as np
import jax.experimental.pallas as pl
import jax.experimental.pallas.tpu as pltpu

S = 2048
D = 1024
DH = 32
WIN = 8
DIL = 2
KS = 4
BL = 128
NB = S // BL
NSTEP = 8
TM = S // NSTEP
CH = D // NSTEP
HALO = 16
F32 = jnp.float32
BF16 = jnp.bfloat16
U32 = jnp.uint32


def _dft_consts():
    n = 2 * BL
    fwd = np.zeros((n, BL), np.float64)
    inv = np.zeros((BL, n), np.float64)
    t = np.arange(BL)
    for g in range(16):
        for r in range(8):
            f = 2 * (8 * g + r)
            ang = 2.0 * np.pi * (f + 0.5) * t / n
            fwd[16 * g + r] = np.cos(ang)
            fwd[16 * g + 8 + r] = -np.sin(ang)
            inv[:, 16 * g + r] = np.cos(ang) * (2.0 / n)
            inv[:, 16 * g + 8 + r] = -np.sin(ang) * (2.0 / n)
    return fwd.astype(np.float32), inv.astype(np.float32)


GATE = True


def _kernel(zero_ref, aq_hbm, ak_hbm, av_hbm, sk_ref, hk_hbm, sd_ref, x_hbm, w_hbm, wo_hbm,
            fwd_ref, inv_ref, out_hbm,
            aq_v, ak_v, av_v, hk_v, x_v, w_v, wo_v, wp, wop, wo_tmp,
            q_s, k_s, v_s, p_s, o_s, kf_s, kv_s, ug_s, y_s, oa_v, ob_v,
            sem_in, sem_w, sem_out):
    lane = jax.lax.broadcasted_iota(jnp.int32, (8, 128), 1)
    row = jax.lax.broadcasted_iota(jnp.int32, (8, 128), 0)
    zero = zero_ref[0]

    def al(i, m):
        return i * m if isinstance(i, int) else pl.multiple_of(i * m, m)

    def in_copy(t, n):
        cs = pl.ds(al(t, CH), CH)
        rs = pl.ds(al(t, TM), TM)
        src, dst = [(ak_hbm.at[:, cs], ak_v), (av_hbm.at[:, cs], av_v), (hk_hbm.at[cs, :], hk_v),
                    (x_hbm.at[rs, :], x_v), (aq_hbm.at[:, cs], aq_v)][n]
        return pltpu.make_async_copy(src, dst.at[t], sem_in.at[t, n])

    def w_copy(n):
        return pltpu.make_async_copy(w_hbm.at[:, pl.ds(n * 128, 128)], w_v.at[n], sem_w.at[n])

    def wo_copy(n):
        return pltpu.make_async_copy(wo_hbm.at[:, pl.ds(n * 128, 128)], wo_v.at[n], sem_w.at[24 + n])

    def copy_a(t):
        return pltpu.make_async_copy(oa_v.at[t], out_hbm.at[:, pl.ds(al(t, CH), CH)], sem_out.at[t, 0])

    def copy_b(t):
        return pltpu.make_async_copy(
            ob_v.at[t + 1], out_hbm.at[pl.ds(al(t, TM), TM), pl.ds(D, D)], sem_out.at[t, 1])

    def xor_select(c, sel):
        for s in range(3):
            bit = (sel & (1 << s)) != 0
            c = [jnp.where(bit, c[i ^ (1 << s)], c[i]) for i in range(8)]
        return c

    def perm_w_sel(sec, rb, RB):
        lane_b = jax.lax.broadcasted_iota(jnp.int32, (RB // 2, 128), 1)
        c = [pltpu.bitcast(w_v[sec * 8 + i, pl.ds(al(rb, RB), RB), :], U32) for i in range(8)]
        c = xor_select(c, lane_b >> 1)
        for i in range(8):
            wp[sec * 8 + i, pl.ds(al(rb, RB // 2), RB // 2), :] = c[i]

    def perm_w_lane(n, j):
        lp = jax.lax.broadcasted_iota(jnp.int32, (D // 2, 128), 1)
        src = (((lp >> 4) & 3) << 5) | ((lp >> 6) << 4) | ((((lp >> 1) & 7) ^ j) << 1) | (lp & 1)
        wp[n] = jnp.take_along_axis(wp[n], src, axis=1)

    def perm_w(sec):
        def body(rb, carry):
            perm_w_sel(sec, rb, 64)
            return carry
        jax.lax.fori_loop(0, D // 64, body, 0)

        def body2(j, carry):
            perm_w_lane(sec * 8 + j, j)
            return carry
        jax.lax.fori_loop(0, 8, body2, 0)

    def perm_wo_c(c):
        wo_tmp[...] = pltpu.bitcast(wo_v[c], U32)
        for mp in range(8):
            m = ((mp & 3) << 1) | (mp >> 2)
            tr = [wo_tmp[pl.ds(m * 8 + j, 8, stride=64), :] for j in range(8)]
            tr = xor_select(tr, row)
            for j in range(8):
                wop[c, pl.ds(j * 64 + mp * 8, 8), :] = tr[j]

    def perm_wo():
        def body(c, carry):
            perm_wo_c(c)
            return carry
        jax.lax.fori_loop(0, 8, body, 0)

    def a_prep(t, j, skt):
        r0 = j * BL
        kf_s[pl.ds(8 + r0, BL), :] = ak_v[t, pl.ds(r0, BL), :].astype(F32)
        ksh = kf_s[pl.ds(8 + r0, BL), :] * skt[0]
        for d in range(1, KS):
            ksh = ksh + kf_s[pl.ds(8 + r0 - d, BL), :] * skt[d]
        kv_s[pl.ds(r0, BL), :] = (ksh * av_v[t, pl.ds(r0, BL), :].astype(F32)).astype(BF16)

    def ug(plane, g, j):
        return (plane * 16 + g) * NB + j

    def a_fwd(t, j, fwd, sd):
        u = jnp.dot(fwd, kv_s[pl.ds(j * BL, BL), :], preferred_element_type=F32)
        h = jax.lax.dot_general(fwd, hk_v[t, :, pl.ds(j * BL, BL)],
                                (((1,), (1,)), ((), ())), preferred_element_type=F32)
        for g in range(16):
            ur, ui = u[16 * g:16 * g + 8], u[16 * g + 8:16 * g + 16]
            ug_s[ug(0, g, j)] = ur + ui
            ug_s[ug(1, g, j)] = ur
            ug_s[ug(2, g, j)] = ui
            hr, hi = h[16 * g:16 * g + 8], h[16 * g + 8:16 * g + 16]
            if j == 0:
                hr = hr + sd
            ug_s[ug(3, g, j)] = hr
            ug_s[ug(4, g, j)] = hi - hr
            ug_s[ug(5, g, j)] = hr + hi

    def a_conv(g):
        prev = None
        for ib in range(4):
            def toep(pl_, acc, sign):
                for jb in range(ib + 1):
                    us = [ug_s[ug(pl_, g, 4 * jb + b)] for b in range(4)]
                    m0 = 4 * (ib - jb)
                    gs = {m: ug_s[ug(3 + pl_, g, m)] for m in range(max(m0 - 3, 0), m0 + 4)}
                    for a in range(4):
                        for b in range(4):
                            m = m0 + a - b
                            if m < 0:
                                continue
                            pr = us[b] * gs[m]
                            if acc[a] is None:
                                acc[a] = pr
                            else:
                                acc[a] = acc[a] + pr if sign > 0 else acc[a] - pr
                return acc
            k1 = toep(0, [None] * 4, 1)
            im = toep(1, list(k1), 1)
            re = toep(2, list(k1), -1)
            for a in range(4):
                if prev is None:
                    yr, yi = re[a], im[a]
                else:
                    yr, yi = re[a] - prev[1], im[a] + prev[0]
                prev = (re[a], im[a])
                y_s[4 * ib + a, pl.ds(16 * g, 16), :] = jnp.concatenate([yr, yi], axis=0).astype(BF16)

    def a_inv(t, i, inv):
        rs = pl.ds(i * BL, BL)
        y = jnp.dot(inv, y_s[i], preferred_element_type=F32)
        oa_v[t, rs, :] = (aq_v[t, rs, :].astype(F32) * y).astype(BF16)

    def b_proj(x, sec, c):
        dst, off = ((q_s, 0), (k_s, HALO), (v_s, HALO))[sec]
        r = jnp.dot(x, pltpu.bitcast(wp[sec * 8 + c], BF16), preferred_element_type=F32)
        dst[c, pl.ds(off, TM), :] = r
        return r[TM - 8:TM]

    cexp = (DH ** -0.5) * math.log2(math.e)
    neg = -1e9 / (DH ** -0.5)
    flip = lane ^ 1

    def b_soft(t, rg):
        r0 = rg * 8
        q = [q_s[c, pl.ds(r0, 8), :] for c in range(8)]
        ls = []
        for w in range(WIN):
            acc = q[0] * k_s[0, pl.ds(HALO + r0 - DIL * w, 8), :]
            for c in range(1, 8):
                acc = acc + q[c] * k_s[c, pl.ds(HALO + r0 - DIL * w, 8), :]
            acc = acc + pltpu.roll(acc, 64, 1)
            acc = acc + jnp.take_along_axis(acc, flip, axis=1)
            if r0 - DIL * w < 0:
                acc = jnp.where(row + (t * TM + r0 - DIL * w) >= 0, acc, neg)
            ls.append(acc)
        m = functools.reduce(jnp.maximum, ls)
        ps = [jnp.exp2((l - m) * cexp) for l in ls]
        inv_den = 1.0 / functools.reduce(lambda a, b: a + b, ps)
        for w in range(WIN):
            p_s[w, pl.ds(r0, 8), :] = ps[w] * inv_den

    def b_av(c):
        for rb in range(TM // 16):
            r0 = rb * 16
            acc = p_s[0, pl.ds(r0, 16), :] * v_s[c, pl.ds(HALO + r0, 16), :]
            for w in range(1, WIN):
                acc = acc + p_s[w, pl.ds(r0, 16), :] * v_s[c, pl.ds(HALO + r0 - DIL * w, 16), :]
            o_s[c, pl.ds(r0, 16), :] = acc.astype(BF16)

    def b_out(t, o, c):
        r = jnp.dot(o, pltpu.bitcast(wop[c], BF16), preferred_element_type=F32)
        ob_v[t + 1, :, pl.ds(c * 128, 128)] = r.astype(BF16)
        return r[TM - 8:TM]

    def load_o():
        return jnp.concatenate([o_s[c] for c in range(8)], axis=1)

    def gate_ug(tok):
        if GATE:
            ug_s[6 * 16 * NB + zero] = tok

    def gate_q(tok):
        if GATE:
            q_s[8 + zero, pl.ds(0, 8), :] = tok

    def gate_kf(tok):
        if GATE:
            kf_s[pl.ds(pl.multiple_of(S + 8 + zero * 8, 8), 8), :] = tok

    def step(t):
        cs = pl.ds(al(t, CH), CH)
        skt_all = sk_ref[:, cs].astype(F32)
        skt = [skt_all[d:d + 1, :] for d in range(KS)]
        sd = sd_ref[:, cs].astype(F32)
        fwd = fwd_ref[...]
        k_s[:, pl.ds(0, HALO), :] = k_s[:, pl.ds(TM, HALO), :]
        v_s[:, pl.ds(0, HALO), :] = v_s[:, pl.ds(TM, HALO), :]
        x = x_v[t]
        for c in range(8):
            a_prep(t, 2 * c, skt)
            a_prep(t, 2 * c + 1, skt)
            tok = b_proj(x, 1, c)
            gate_kf(tok)
            a_fwd(t, 2 * c, fwd, sd)
            a_fwd(t, 2 * c + 1, fwd, sd)
        conv_sched = iter(range(16))
        for c in range(8):
            a_conv(next(conv_sched))
            tok = b_proj(x, 0, c)
            gate_ug(tok)
        o = load_o()
        for c in range(8):
            for rg in range(4):
                b_soft(t, c * 4 + rg)
            if c % 4 == 1:
                a_conv(next(conv_sched))
            tok = b_out(t - 1, o, c)
            gate_ug(tok)
            gate_q(tok)
        for c in range(8):
            if c % 4 != 3:
                a_conv(next(conv_sched))
            tok = b_proj(x, 2, c)
            gate_ug(tok)
            b_av(c)
        inv = inv_ref[...]
        for i in range(NB):
            a_inv(t, i, inv)

    for n in range(24):
        w_copy(n).start()
    for n in range(8):
        wo_copy(n).start()
    for n in range(5):
        in_copy(0, n).start()
    k_s[:, pl.ds(TM, HALO), :] = jnp.zeros((8, HALO, 128), F32)
    v_s[:, pl.ds(TM, HALO), :] = jnp.zeros((8, HALO, 128), F32)
    kf_s[pl.ds(0, 8), :] = jnp.zeros((8, 128), F32)
    o_s[...] = jnp.zeros(o_s.shape, BF16)
    for sec in range(3):
        for n in range(8):
            w_copy(sec * 8 + n).wait()
        perm_w(sec)
    for n in range(8):
        wo_copy(n).wait()
    perm_wo()

    def loop(t, carry):
        for n in range(5):
            in_copy(t, n).wait()

        @pl.when(t + 1 < NSTEP)
        def _():
            for n in range(5):
                in_copy(t + 1, n).start()
        step(t)
        copy_a(t).start()

        @pl.when(t > 0)
        def _():
            copy_b(t - 1).start()
        return carry
    jax.lax.fori_loop(0, NSTEP, loop, 0)

    o = load_o()
    for c in range(8):
        b_out(NSTEP - 1, o, c)
    copy_b(NSTEP - 1).start()
    for t in range(NSTEP):
        copy_a(t).wait()
        copy_b(t).wait()


@jax.jit
def pallas_concat_heads__ssm_conv_h3__sliding_local_dilated__prompt_kernel(
    A_q, A_k, A_v, A_shift_k, A_ssm_k, A_ssm_D, B_x, B_wqkv, B_wo,
):
    fwd, inv = _dft_consts()
    fwd = jnp.asarray(fwd, BF16)
    inv = jnp.asarray(inv, BF16)
    hbm = pl.BlockSpec(memory_space=pl.ANY)
    vmem = pl.BlockSpec(memory_space=pltpu.VMEM)
    smem = pl.BlockSpec(memory_space=pltpu.SMEM)
    out = pl.pallas_call(
        _kernel,
        in_specs=[smem, hbm, hbm, hbm, vmem, hbm, vmem, hbm, hbm, hbm, vmem, vmem],
        out_specs=hbm,
        out_shape=jax.ShapeDtypeStruct((S, 2 * D), BF16),
        scratch_shapes=[
            pltpu.VMEM((NSTEP, S, CH), BF16),
            pltpu.VMEM((NSTEP, S, CH), BF16),
            pltpu.VMEM((NSTEP, S, CH), BF16),
            pltpu.VMEM((NSTEP, CH, S), BF16),
            pltpu.VMEM((NSTEP, TM, D), BF16),
            pltpu.VMEM((24, D, 128), BF16),
            pltpu.VMEM((8, D, 128), BF16),
            pltpu.VMEM((24, D // 2, 128), U32),
            pltpu.VMEM((8, D // 2, 128), U32),
            pltpu.VMEM((D // 2, 128), U32),
            pltpu.VMEM((9, TM, 128), F32),
            pltpu.VMEM((8, TM + HALO, 128), F32),
            pltpu.VMEM((8, TM + HALO, 128), F32),
            pltpu.VMEM((WIN, TM, 128), F32),
            pltpu.VMEM((8, TM, 128), BF16),
            pltpu.VMEM((S + 16, 128), F32),
            pltpu.VMEM((S, 128), BF16),
            pltpu.VMEM((6 * 16 * NB + 1, 8, 128), F32),
            pltpu.VMEM((NB, 2 * BL, 128), BF16),
            pltpu.VMEM((NSTEP, S, CH), BF16),
            pltpu.VMEM((NSTEP + 1, TM, D), BF16),
            pltpu.SemaphoreType.DMA((NSTEP, 5)),
            pltpu.SemaphoreType.DMA((32,)),
            pltpu.SemaphoreType.DMA((NSTEP, 2)),
        ],
        compiler_params=pltpu.CompilerParams(vmem_limit_bytes=100 * 1024 * 1024),
    )(jnp.zeros((1,), jnp.int32), A_q.reshape(S, D), A_k.reshape(S, D), A_v.reshape(S, D),
      A_shift_k.T, A_ssm_k, A_ssm_D.reshape(1, D),
      B_x.reshape(S, D), B_wqkv, B_wo, fwd, inv)
    return out.reshape(1, S, 2 * D)
```

```python
import functools
import math

import jax
import jax.numpy as jnp
import numpy as np
import jax.experimental.pallas as pl
import jax.experimental.pallas.tpu as pltpu

S = 2048
D = 1024
DH = 32
WIN = 8
DIL = 2
KS = 4
BL = 128
NB = S // BL
NSTEP = 8
TM = S // NSTEP
CH = D // NSTEP
HALO = 16
F32 = jnp.float32
BF16 = jnp.bfloat16
U32 = jnp.uint32


def _dft_consts():
    n = 2 * BL
    fwd = np.zeros((n, BL), np.float64)
    inv = np.zeros((BL, n), np.float64)
    t = np.arange(BL)
    for g in range(16):
        for r in range(8):
            f = 2 * (8 * g + r)
            ang = 2.0 * np.pi * (f + 0.5) * t / n
            fwd[16 * g + r] = np.cos(ang)
            fwd[16 * g + 8 + r] = -np.sin(ang)
            inv[:, 16 * g + r] = np.cos(ang) * (2.0 / n)
            inv[:, 16 * g + 8 + r] = -np.sin(ang) * (2.0 / n)
    return fwd.astype(np.float32), inv.astype(np.float32)


import os
NZ = 64
LEAD = int(os.environ.get('LEAD', 8))
FIN = int(os.environ.get('FIN', 44))
TAIL = int(os.environ.get('TAIL', 12))
CONV_W = [3] * 8 + [8] * 15 + [3]
PRO_CONV = 12


def _pack_rows(a):
    b = np.asarray(a, dtype=jnp.bfloat16).view(np.uint16).astype(np.uint32)
    return (b[0::2] | (b[1::2] << 16))[None]


def _kernel(zero_ref, aq_hbm, ak_hbm, av_hbm, sk_ref, hk_hbm, sd_ref, x_hbm, w_hbm, wo_hbm,
            fwd_ref, inv_ref, out_hbm,
            aq_v, ak_v, av_v, hk_v, x_v, w_v, wo_v, wp, wo_tmp,
            xu, ou, acc_s, q_s, k_s, v_s, p_s, o_s, kf_s, kv_s, ug_s, y_s, oa_v, ob_v,
            sem_in, sem_w, sem_out):
    lane = jax.lax.broadcasted_iota(jnp.int32, (8, 128), 1)
    row = jax.lax.broadcasted_iota(jnp.int32, (8, 128), 0)
    zero = zero_ref[0]
    zcount = [0]
    P = functools.partial

    def z():
        zcount[0] = zcount[0] % (NZ - 1) + 1
        return zero_ref[zcount[0]]

    def al(i, m):
        return i * m if isinstance(i, int) else pl.multiple_of(i * m, m)

    def in_copy(t, n):
        cs = pl.ds(al(t, CH), CH)
        rs = pl.ds(al(t, TM), TM)
        if n == 0:
            src, dst = ak_hbm.at[:, cs], ak_v
        elif n == 1:
            src, dst = av_hbm.at[:, cs], av_v
        elif n == 2:
            src, dst = hk_hbm.at[cs, :], hk_v
        elif n == 3:
            src, dst = x_hbm.at[rs, :], x_v
        else:
            src, dst = aq_hbm.at[:, cs], aq_v
        return pltpu.make_async_copy(src, dst.at[t], sem_in.at[t, n])

    def w_copy(n):
        return pltpu.make_async_copy(w_hbm.at[:, pl.ds(n * 128, 128)], w_v.at[n], sem_w.at[n])

    def wo_copy(n):
        return pltpu.make_async_copy(wo_hbm.at[:, pl.ds(n * 128, 128)], wo_v.at[n], sem_w.at[24 + n])

    def copy_a(t):
        return pltpu.make_async_copy(oa_v.at[t], out_hbm.at[:, pl.ds(al(t, CH), CH)], sem_out.at[t, 0])

    def copy_b(t):
        return pltpu.make_async_copy(
            ob_v.at[t], out_hbm.at[pl.ds(al(t, TM), TM), pl.ds(D, D)], sem_out.at[t, 1])

    def copy_b_last(n):
        t = NSTEP - 1
        return pltpu.make_async_copy(
            ob_v.at[t, :, pl.ds(n * 256, 256)],
            out_hbm.at[pl.ds(t * TM, TM), pl.ds(D + n * 256, 256)], sem_out.at[t, 1 + n])

    def xor_select(c, sel):
        for s in range(3):
            bit = (sel & (1 << s)) != 0
            c = [jnp.where(bit, c[i ^ (1 << s)], c[i]) for i in range(8)]
        return c

    def tsum(vals):
        return functools.reduce(lambda a, b: a + b, vals)

    def lane_src(j):
        return (((lane >> 4) & 3) << 5) | ((lane >> 6) << 4) | ((((lane >> 1) & 7) ^ j) << 1) | (lane & 1)

    def perm_w(sec, rb):
        c = [pltpu.bitcast(w_v[sec * 8 + i, pl.ds(rb * 16, 16), :], U32) for i in range(8)]
        c = xor_select(c, lane >> 1)
        for j in range(8):
            c[j] = jnp.take_along_axis(c[j], lane_src(j), axis=1)
            wp[sec * 8 + j, pl.ds(rb * 8, 8), :] = c[j]

    def perm_wo(c):
        wo_tmp[c] = pltpu.bitcast(wo_v[c], U32)
        for mp in range(8):
            m = ((mp & 3) << 1) | (mp >> 2)
            tr = [wo_tmp[c, pl.ds(m * 8 + j, 8, stride=64), :] for j in range(8)]
            tr = xor_select(tr, row)
            for j in range(8):
                wp[24 + c, pl.ds(j * 64 + mp * 8, 8), :] = tr[j]

    def a_prep(t, r0, n, skt):
        kf_s[pl.ds(8 + r0, n), :] = ak_v[t, pl.ds(r0, n), :].astype(F32)
        ksh = kf_s[pl.ds(8 + r0, n), :] * skt[0]
        for d in range(1, KS):
            ksh = ksh + kf_s[pl.ds(8 + r0 - d, n), :] * skt[d]
        kv_s[pl.ds(r0, n), :] = (ksh * av_v[t, pl.ds(r0, n), :].astype(F32)).astype(BF16)

    def prep_units(t, j, skt):
        return [('prep', 48, P(a_prep, t, j * BL + r, 32, skt)) for r in range(0, BL, 32)]

    def slabs(r):
        return [r[i:i + 8] for i in range(0, r.shape[0], 16)]

    def ug(plane, g, j):
        return (plane * 16 + g) * NB + j

    def a_fwd(t, j, sd):
        fwd = pltpu.bitcast(fwd_ref[z()], BF16)
        u = jnp.dot(fwd, kv_s[pl.ds(j * BL, BL), :], preferred_element_type=F32)
        fwd = pltpu.bitcast(fwd_ref[z()], BF16)
        h = jax.lax.dot_general(fwd, hk_v[t, :, pl.ds(j * BL, BL)],
                                (((1,), (1,)), ((), ())), preferred_element_type=F32)
        for g in range(16):
            ur, ui = u[16 * g:16 * g + 8], u[16 * g + 8:16 * g + 16]
            ug_s[ug(0, g, j)] = ur + ui
            ug_s[ug(1, g, j)] = ur
            ug_s[ug(2, g, j)] = ui
            hr, hi = h[16 * g:16 * g + 8], h[16 * g + 8:16 * g + 16]
            if j == 0:
                hr = hr + sd
            ug_s[ug(3, g, j)] = hr
            ug_s[ug(4, g, j)] = hi - hr
            ug_s[ug(5, g, j)] = hr + hi
        return slabs(u)

    def conv_units(g):
        st = {'prev': None}

        def toep(ib, pl_):
            zi = z()
            acc = [None] * 4 if pl_ == 0 else list(st[0])
            gs = {}
            for jb in range(ib + 1):
                us = [ug_s[zi + ug(pl_, g, 4 * jb + b)] for b in range(4)]
                m0 = 4 * (ib - jb)
                gs = {m: gs[m] if m in gs else ug_s[zi + ug(3 + pl_, g, m)]
                      for m in range(max(m0 - 3, 0), m0 + 4)}
                for a in range(4):
                    for b in range(4):
                        m = m0 + a - b
                        if m < 0:
                            continue
                        pr = us[b] * gs[m]
                        if acc[a] is None:
                            acc[a] = pr
                        else:
                            acc[a] = acc[a] + pr if pl_ < 2 else acc[a] - pr
            st[pl_] = acc
            if pl_ == 2:
                im, re = st[1], st[2]
                for a in range(4):
                    prev = st['prev']
                    if prev is None:
                        yr, yi = re[a], im[a]
                    else:
                        yr, yi = re[a] - prev[1], im[a] + prev[0]
                    st['prev'] = (re[a], im[a])
                    y_s[4 * ib + a, pl.ds(16 * g, 16), :] = jnp.concatenate([yr, yi], axis=0).astype(BF16)
        return [('conv', 20 + 32 * ib + (12 if pl_ == 2 else 0), P(toep, ib, pl_))
                for ib in range(4) for pl_ in range(3)]

    def a_conv(g):
        for _, _, fn in conv_units(g):
            fn()

    def a_inv(t, i):
        rs = pl.ds(i * BL, BL)
        inv = pltpu.bitcast(inv_ref[z()], BF16)
        y = jnp.dot(inv, y_s[i], preferred_element_type=F32)
        r = aq_v[t, rs, :].astype(F32) * y
        oa_v[t, rs, :] = r.astype(BF16)
        return slabs(y)

    def stage_x(t, slot):
        xu[slot] = pltpu.bitcast(x_v[t], U32)

    def mm2(lhs, li, wi, part, pi, off):
        h = D // 2
        x = pltpu.bitcast(lhs[li + z(), :, pl.ds(0, h)], BF16)
        r1 = jnp.dot(x, pltpu.bitcast(wp[wi, pl.ds(0, h // 2), :], BF16), preferred_element_type=F32)
        part[pi, pl.ds(off, TM), :] = r1
        x = pltpu.bitcast(lhs[li + z(), :, pl.ds(h, h)], BF16)
        r2 = jnp.dot(x, pltpu.bitcast(wp[wi, pl.ds(h // 2, h // 2), :], BF16), preferred_element_type=F32)
        r = part[pi + z(), pl.ds(off, TM), :] + r2
        return r, slabs(r1) + slabs(r2)

    def b_proj(slot, sec, c):
        dst, off = ((q_s, 0), (k_s, HALO), (v_s, HALO))[sec]
        r, toks = mm2(xu, slot, sec * 8 + c, dst, c, off)
        dst[c, pl.ds(off, TM), :] = r
        return toks

    cexp = (DH ** -0.5) * math.log2(math.e)
    neg = -1e9 / (DH ** -0.5)
    flip = lane ^ 1

    def soft_units(t, rg):
        r0 = rg * 8
        st = {'ls': []}

        def logits(ws):
            zi = z()
            q = [q_s[zi + c, pl.ds(r0, 8), :] for c in range(8)]
            for w in ws:
                acc = q[0] * k_s[zi, pl.ds(HALO + r0 - DIL * w, 8), :]
                for c in range(1, 8):
                    acc = acc + q[c] * k_s[zi + c, pl.ds(HALO + r0 - DIL * w, 8), :]
                acc = acc + pltpu.roll(acc, 64, 1)
                acc = acc + jnp.take_along_axis(acc, flip, axis=1)
                if r0 - DIL * w < 0 and not (isinstance(t, int) and t > 0):
                    acc = jnp.where(row + (t * TM + r0 - DIL * w) >= 0, acc, neg)
                st['ls'].append(acc)
            if len(st['ls']) == WIN:
                ls = st['ls']
                m = functools.reduce(jnp.maximum, ls)
                ps = [jnp.exp2((l - m) * cexp) for l in ls]
                inv_den = 1.0 / tsum(ps)
                for w in range(WIN):
                    p_s[w, pl.ds(r0, 8), :] = ps[w] * inv_den
        return [('soft', 68, P(logits, range(0, 4))), ('soft', 108, P(logits, range(4, 8)))]

    def av_units(c):
        def av(rbs):
            for rb in rbs:
                r0 = rb * 16
                zi = z()
                acc = p_s[zi, pl.ds(r0, 16), :] * v_s[zi + c, pl.ds(HALO + r0, 16), :]
                for w in range(1, WIN):
                    acc = acc + p_s[zi + w, pl.ds(r0, 16), :] * v_s[zi + c, pl.ds(HALO + r0 - DIL * w, 16), :]
                o_s[c, pl.ds(r0, 16), :] = acc.astype(BF16)
            if rbs[-1] == TM // 16 - 1:
                ou[0, :, pl.ds(c * 128, 128)] = pltpu.bitcast(o_s[c + z()], U32)
        return [('av', 64, P(av, (rb, rb + 1))) for rb in range(0, TM // 16, 2)]

    def b_out(t, c):
        r, toks = mm2(ou, 0, 24 + c, acc_s, c % 2, 0)
        ob_v[t, :, pl.ds(c * 128, 128)] = r.astype(BF16)
        return toks

    def gate(kind, tok):
        if kind == 'conv':
            ug_s[6 * 16 * NB + zero] = tok
        elif kind == 'soft':
            q_s[8 + zero, pl.ds(0, 8), :] = tok
        elif kind == 'av':
            p_s[8 + zero, pl.ds(0, 8), :] = tok
        elif kind == 'prep':
            kf_s[pl.ds(pl.multiple_of(S + 8 + zero * 8, 8), 8), :] = tok

    def a_consts(t):
        cs = pl.ds(al(t, CH), CH)
        skt_all = sk_ref[:, cs].astype(F32)
        return [skt_all[d:d + 1, :] for d in range(KS)], sd_ref[:, cs].astype(F32)

    def halo(ref):
        ref[:, pl.ds(0, HALO), :] = ref[:, pl.ds(TM, HALO), :]

    def pace(toks, units, lead=0):
        total = sum(u[1] for u in units)
        done = 0
        last = {}
        for kind, cost, fn in units:
            i = (len(toks) + lead) * done // total - lead
            if i >= 0 and last.get(kind) != i:
                gate(kind, toks[i])
                last[kind] = i
            fn()
            done += cost

    def merge(*lists):
        items = []
        for l in lists:
            tot = sum(u[1] for u in l)
            acc = 0
            for u in l:
                items.append((acc / tot, len(items), u))
                acc += u[1]
        return [u for _, _, u in sorted(items, key=lambda x: x[:2])]

    for n in range(4):
        in_copy(0, n).start()
    for sec in (1, 0, 2):
        for n in range(8):
            w_copy(sec * 8 + n).start()
    for n in range(8):
        wo_copy(n).start()
    in_copy(0, 4).start()
    for n in range(4):
        in_copy(1, n).start()
    k_s[:, pl.ds(0, HALO), :] = jnp.zeros((8, HALO, 128), F32)
    v_s[:, pl.ds(TM, HALO), :] = jnp.zeros((8, HALO, 128), F32)
    kf_s[pl.ds(0, 8), :] = jnp.zeros((8, 128), F32)
    for n in range(3):
        in_copy(0, n).wait()
    skt, sd = a_consts(0)
    for j in range(NB):
        a_prep(0, j * BL, BL, skt)
        a_fwd(0, j, sd)
    for g in range(PRO_CONV):
        a_conv(g)
    for n in range(8):
        w_copy(8 + n).wait()
    for rb in range(64):
        perm_w(1, rb)
    in_copy(0, 3).wait()
    for n in range(8):
        w_copy(n).wait()
    stage_x(0, 0)
    conv_sched = iter(range(PRO_CONV, 16))
    for c in range(8):
        b_proj(0, 1, c)
        for rb in range(8):
            perm_w(0, 8 * c + rb)
    for n in range(8):
        w_copy(16 + n).wait()
    for c in range(8):
        b_proj(0, 0, c)
        for rb in range(8):
            perm_w(2, 8 * c + rb)
        g = next(conv_sched, None)
        if g is not None:
            a_conv(g)
    for n in range(8):
        wo_copy(n).wait()
    for c in range(8):
        perm_wo(c)

    def loop(t, carry):
        in_copy(t, 4).wait()
        for n in range(4):
            in_copy(t + 1, n).wait()
        in_copy(t + 1, 4).start()

        @pl.when(t + 2 < NSTEP)
        def _():
            for n in range(4):
                in_copy(t + 2, n).start()

        halo(v_s)
        skt, sd = a_consts(t + 1)
        stage_x(t + 1, (t + 1) % 2)

        for u in prep_units(t + 1, 0, skt) + prep_units(t + 1, 1, skt):
            u[2]()
        for c in range(8):
            toks = b_proj(t % 2, 2, c)
            toks += a_inv(t, 2 * c)
            a_inv(t, 2 * c + 1)
            toks += a_fwd(t + 1, 2 * c, sd)
            a_fwd(t + 1, 2 * c + 1, sd)
            soft = [u for rg in range(4 * c, 4 * c + 4) for u in soft_units(t, rg)]
            if c < 7:
                pace(toks, merge(soft, prep_units(t + 1, 2 * c + 2, skt) + prep_units(t + 1, 2 * c + 3, skt)),
                     LEAD if c == 0 else 0)
            else:
                pace(toks[:FIN], soft)
        halo(k_s)
        conv = [u for g in range(16) for u in conv_units(g)]
        ctot = sum(u[1] for u in conv)
        cdone = 0
        for k in range(24):
            ph, c = divmod(k, 8)
            toks = b_out(t, c) if ph == 2 else b_proj((t + 1) % 2, 1 - ph, c)
            mine = []
            while conv and cdone < ctot * sum(CONV_W[:k + 1]) / sum(CONV_W):
                cdone += conv[0][1]
                mine.append(conv.pop(0))
            units = merge(mine, av_units(c)) if ph == 0 and mine else (av_units(c) if ph == 0 else mine)
            if units:
                pace(toks[:TAIL] if k == 23 else toks, units)
        copy_a(t).start()
        copy_b(t).start()
        return carry
    jax.lax.fori_loop(0, NSTEP - 1, loop, 0)

    t = NSTEP - 1
    in_copy(t, 4).wait()
    halo(v_s)
    for c in range(8):
        toks = b_proj(t % 2, 2, c)
        if c < 5:
            pace(toks, [u for rg in range(32) if rg * 5 // 32 == c for u in soft_units(t, rg)],
                 LEAD if c == 0 else 0)
        else:
            pace(toks, [u for cc in ((0, 1), (2, 3), (4, 5))[c - 5] for u in av_units(cc)])
    toks = []
    for i in range(NB):
        tk = a_inv(t, i)
        if i % 2 == 0:
            toks += tk
    pace(toks[:40], av_units(6) + av_units(7))
    copy_a(t).start()
    for c in range(8):
        b_out(t, c)
        if c % 2 == 1:
            copy_b_last(c // 2).start()
    for s in range(NSTEP - 1):
        copy_a(s).wait()
        copy_b(s).wait()
    copy_a(t).wait()
    for n in range(4):
        copy_b_last(n).wait()


@jax.jit
def pallas_concat_heads__ssm_conv_h3__sliding_local_dilated__prompt_kernel(
    A_q, A_k, A_v, A_shift_k, A_ssm_k, A_ssm_D, B_x, B_wqkv, B_wo,
):
    fwd, inv = _dft_consts()
    fwd = jnp.asarray(_pack_rows(fwd))
    inv = jnp.asarray(_pack_rows(inv))
    hbm = pl.BlockSpec(memory_space=pl.ANY)
    vmem = pl.BlockSpec(memory_space=pltpu.VMEM)
    smem = pl.BlockSpec(memory_space=pltpu.SMEM)
    out = pl.pallas_call(
        _kernel,
        in_specs=[smem, hbm, hbm, hbm, vmem, hbm, vmem, hbm, hbm, hbm, vmem, vmem],
        out_specs=hbm,
        out_shape=jax.ShapeDtypeStruct((S, 2 * D), BF16),
        scratch_shapes=[
            pltpu.VMEM((NSTEP, S, CH), BF16),
            pltpu.VMEM((NSTEP, S, CH), BF16),
            pltpu.VMEM((NSTEP, S, CH), BF16),
            pltpu.VMEM((NSTEP, CH, S), BF16),
            pltpu.VMEM((NSTEP, TM, D), BF16),
            pltpu.VMEM((24, D, 128), BF16),
            pltpu.VMEM((8, D, 128), BF16),
            pltpu.VMEM((32, D // 2, 128), U32),
            pltpu.VMEM((8, D // 2, 128), U32),
            pltpu.VMEM((2, TM // 2, D), U32),
            pltpu.VMEM((1, TM // 2, D), U32),
            pltpu.VMEM((2, TM, 128), F32),
            pltpu.VMEM((9, TM, 128), F32),
            pltpu.VMEM((8, TM + HALO, 128), F32),
            pltpu.VMEM((8, TM + HALO, 128), F32),
            pltpu.VMEM((WIN + 1, TM, 128), F32),
            pltpu.VMEM((8, TM, 128), BF16),
            pltpu.VMEM((S + 16, 128), F32),
            pltpu.VMEM((S, 128), BF16),
            pltpu.VMEM((6 * 16 * NB + 1, 8, 128), F32),
            pltpu.VMEM((NB, 2 * BL, 128), BF16),
            pltpu.VMEM((NSTEP, S, CH), BF16),
            pltpu.VMEM((NSTEP, TM, D), BF16),
            pltpu.SemaphoreType.DMA((NSTEP, 5)),
            pltpu.SemaphoreType.DMA((32,)),
            pltpu.SemaphoreType.DMA((NSTEP, 5)),
        ],
        compiler_params=pltpu.CompilerParams(vmem_limit_bytes=100 * 1024 * 1024),
    )(jnp.zeros((NZ,), jnp.int32), A_q.reshape(S, D), A_k.reshape(S, D), A_v.reshape(S, D),
      A_shift_k.T, A_ssm_k, A_ssm_D.reshape(1, D),
      B_x.reshape(S, D), B_wqkv, B_wo, fwd, inv)
    return out.reshape(1, S, 2 * D)
```

```python
import functools
import math

import jax
import jax.numpy as jnp
import numpy as np
import jax.experimental.pallas as pl
import jax.experimental.pallas.tpu as pltpu

S = 2048
D = 1024
DH = 32
WIN = 8
DIL = 2
KS = 4
BL = 128
NB = S // BL
NSTEP = 8
TM = S // NSTEP
CH = D // NSTEP
HALO = 16
F32 = jnp.float32
BF16 = jnp.bfloat16
U32 = jnp.uint32


def _dft_consts():
    n = 2 * BL
    fwd = np.zeros((n, BL), np.float64)
    inv = np.zeros((BL, n), np.float64)
    t = np.arange(BL)
    for g in range(16):
        for r in range(8):
            f = 2 * (8 * g + r)
            ang = 2.0 * np.pi * (f + 0.5) * t / n
            fwd[16 * g + r] = np.cos(ang)
            fwd[16 * g + 8 + r] = -np.sin(ang)
            inv[:, 16 * g + r] = np.cos(ang) * (2.0 / n)
            inv[:, 16 * g + 8 + r] = -np.sin(ang) * (2.0 / n)
    return fwd.astype(np.float32), inv.astype(np.float32)


import os
NZ = 64
NTINY = 6
LEAD = int(os.environ.get('LEAD', 8))
FIN = int(os.environ.get('FIN', 44))
TAIL = int(os.environ.get('TAIL', 12))
CONV_W = [3] * 8 + [8] * 15 + [3]
CONV_W1 = [4] * 8 + [6] * 8 + [9] * 7 + [3]
PRO_CONV = int(os.environ.get('PRO_CONV', 12))
PRO_WQ = int(os.environ.get('PRO_WQ', 8))


def _pack_rows(a):
    b = np.asarray(a, dtype=jnp.bfloat16).view(np.uint16).astype(np.uint32)
    return (b[0::2] | (b[1::2] << 16))[None]


def _kernel(zero_ref, aq_hbm, ak_hbm, av_hbm, sk_ref, hk_hbm, sd_ref, x_hbm, w_hbm, wo_hbm,
            fwd_ref, inv_ref, out_hbm,
            aq_v, ak_v, av_v, hk_v, x_v, w_v, wp, wt_a, wt_b,
            xu, ou, acc_s, q_s, k_s, v_s, p_s, o_s, kf_s, kv_s, ug_s, y_s, oa_v, ob_v, tiny_v,
            sem_in, sem_w, sem_out):
    lane = jax.lax.broadcasted_iota(jnp.int32, (8, 128), 1)
    row = jax.lax.broadcasted_iota(jnp.int32, (8, 128), 0)
    zero = zero_ref[0]
    zcount = [0]
    P = functools.partial

    def z():
        zcount[0] = zcount[0] % (NZ - 1) + 1
        return zero_ref[zcount[0]]

    def al(i, m):
        return i * m if isinstance(i, int) else pl.multiple_of(i * m, m)

    def in_copy(t, n):
        cs = pl.ds(al(t, CH), CH)
        rs = pl.ds(al(t, TM), TM)
        if n == 0:
            src, dst = ak_hbm.at[:, cs], ak_v
        elif n == 1:
            src, dst = av_hbm.at[:, cs], av_v
        elif n == 2:
            src, dst = hk_hbm.at[cs, :], hk_v
        elif n == 3:
            src, dst = x_hbm.at[rs, :], x_v
        else:
            src, dst = aq_hbm.at[:, cs], aq_v
        return pltpu.make_async_copy(src, dst.at[t], sem_in.at[t, n])

    def w_copy(n):
        return pltpu.make_async_copy(w_hbm.at[:, pl.ds(n * 128, 128)], w_v.at[n], sem_w.at[n])

    def wo_copy(n):
        return pltpu.make_async_copy(wo_hbm.at[:, pl.ds(n * 128, 128)], w_v.at[24 + n], sem_w.at[24 + n])

    def copy_a(t):
        return pltpu.make_async_copy(oa_v.at[t], out_hbm.at[:, pl.ds(al(t, CH), CH)], sem_out.at[t, 0])

    def copy_b(t):
        return pltpu.make_async_copy(
            ob_v.at[t], out_hbm.at[pl.ds(al(t, TM), TM), pl.ds(D, D)], sem_out.at[t, 1])

    def copy_b_last(n):
        t = NSTEP - 1
        return pltpu.make_async_copy(
            ob_v.at[t, :, pl.ds(n * 256, 256)],
            out_hbm.at[pl.ds(t * TM, TM), pl.ds(D + n * 256, 256)], sem_out.at[t, 1 + n])

    def xor_select(c, sel):
        for s in range(3):
            bit = (sel & (1 << s)) != 0
            c = [jnp.where(bit, c[i ^ (1 << s)], c[i]) for i in range(8)]
        return c

    def tsum(vals):
        return functools.reduce(lambda a, b: a + b, vals)

    def lane_src(j):
        return (((lane >> 4) & 3) << 5) | ((lane >> 6) << 4) | ((((lane >> 1) & 7) ^ j) << 1) | (lane & 1)

    def wtmp(sec):
        return (wt_b, wt_a, wt_a)[sec], ('wtb', 'wta', 'wta')[sec]

    def sel_units(sec):
        wt, _ = wtmp(sec)

        def sel(rb):
            c = [pltpu.bitcast(w_v[sec * 8 + i, pl.ds(rb * 16, 16), :], U32) for i in range(8)]
            c = xor_select(c, lane >> 1)
            for j in range(8):
                wt[j, pl.ds(rb * 8, 8), :] = c[j]
        return [('wv', 32, P(sel, rb)) for rb in range(64)]

    def lane_units(sec, j):
        wt, kind = wtmp(sec)

        def lanes(rb):
            zi = z()
            for r in range(rb * 64, rb * 64 + 64, 8):
                wp[sec * 8 + j, pl.ds(r, 8), :] = jnp.take_along_axis(
                    wt[zi + j, pl.ds(r, 8), :], lane_src(j), axis=1)
        return [(kind, 32, P(lanes, rb)) for rb in range(8)]

    def wo_units(c):
        def rows(mp):
            m = ((mp & 3) << 1) | (mp >> 2)
            tr = [pltpu.bitcast(w_v[24 + c, pl.ds(r * 128 + m * 16, 16), :], U32) for r in range(8)]
            tr = xor_select(tr, row)
            for j in range(8):
                wp[24 + c, pl.ds(j * 64 + mp * 8, 8), :] = (
                    jnp.take_along_axis(tr[j], row ^ j, axis=0) if j else tr[j])
        return [('wv', 40, P(rows, mp)) for mp in range(8)]

    def a_prep(t, r0, n, skt):
        kf_s[pl.ds(8 + r0, n), :] = ak_v[t, pl.ds(r0, n), :].astype(F32)
        ksh = kf_s[pl.ds(8 + r0, n), :] * skt[0]
        for d in range(1, KS):
            ksh = ksh + kf_s[pl.ds(8 + r0 - d, n), :] * skt[d]
        kv_s[pl.ds(r0, n), :] = (ksh * av_v[t, pl.ds(r0, n), :].astype(F32)).astype(BF16)

    def prep_units(t, j, skt):
        return [('prep', 48, P(a_prep, t, j * BL + r, 32, skt)) for r in range(0, BL, 32)]

    def slabs(r):
        return [r[i:i + 8] for i in range(0, r.shape[0], 16)]

    def ug(plane, g, j):
        return (plane * 16 + g) * NB + j

    def a_fwd(t, j, sd):
        fwd = pltpu.bitcast(fwd_ref[z()], BF16)
        u = jnp.dot(fwd, kv_s[pl.ds(j * BL, BL), :], preferred_element_type=F32)
        fwd = pltpu.bitcast(fwd_ref[z()], BF16)
        h = jax.lax.dot_general(fwd, hk_v[t, :, pl.ds(j * BL, BL)],
                                (((1,), (1,)), ((), ())), preferred_element_type=F32)
        for g in range(16):
            ur, ui = u[16 * g:16 * g + 8], u[16 * g + 8:16 * g + 16]
            ug_s[ug(0, g, j)] = ur + ui
            ug_s[ug(1, g, j)] = ur
            ug_s[ug(2, g, j)] = ui
            hr, hi = h[16 * g:16 * g + 8], h[16 * g + 8:16 * g + 16]
            if j == 0:
                hr = hr + sd
            ug_s[ug(3, g, j)] = hr
            ug_s[ug(4, g, j)] = hi - hr
            ug_s[ug(5, g, j)] = hr + hi
        return slabs(u)

    def conv_units(g):
        st = {'prev': None}

        def toep(ib, pl_):
            zi = z()
            acc = [None] * 4 if pl_ == 0 else list(st[0])
            gs = {}
            for jb in range(ib + 1):
                us = [ug_s[zi + ug(pl_, g, 4 * jb + b)] for b in range(4)]
                m0 = 4 * (ib - jb)
                gs = {m: gs[m] if m in gs else ug_s[zi + ug(3 + pl_, g, m)]
                      for m in range(max(m0 - 3, 0), m0 + 4)}
                for a in range(4):
                    for b in range(4):
                        m = m0 + a - b
                        if m < 0:
                            continue
                        pr = us[b] * gs[m]
                        if acc[a] is None:
                            acc[a] = pr
                        else:
                            acc[a] = acc[a] + pr if pl_ < 2 else acc[a] - pr
            st[pl_] = acc
            if pl_ == 2:
                im, re = st[1], st[2]
                for a in range(4):
                    prev = st['prev']
                    if prev is None:
                        yr, yi = re[a], im[a]
                    else:
                        yr, yi = re[a] - prev[1], im[a] + prev[0]
                    st['prev'] = (re[a], im[a])
                    y_s[4 * ib + a, pl.ds(16 * g, 16), :] = jnp.concatenate([yr, yi], axis=0).astype(BF16)
        return [('conv', 20 + 32 * ib + (12 if pl_ == 2 else 0), P(toep, ib, pl_))
                for ib in range(4) for pl_ in range(3)]

    def a_conv(g):
        for _, _, fn in conv_units(g):
            fn()

    def a_inv(t, i):
        rs = pl.ds(i * BL, BL)
        inv = pltpu.bitcast(inv_ref[z()], BF16)
        y = jnp.dot(inv, y_s[i], preferred_element_type=F32)
        r = aq_v[t, rs, :].astype(F32) * y
        oa_v[t, rs, :] = r.astype(BF16)
        return slabs(y)

    def stage_x(t, slot):
        xu[slot] = pltpu.bitcast(x_v[t], U32)

    def mm2(lhs, li, wi, part, pi, off):
        h = D // 2
        x = pltpu.bitcast(lhs[li + z(), :, pl.ds(0, h)], BF16)
        r1 = jnp.dot(x, pltpu.bitcast(wp[wi, pl.ds(0, h // 2), :], BF16), preferred_element_type=F32)
        part[pi, pl.ds(off, TM), :] = r1
        x = pltpu.bitcast(lhs[li + z(), :, pl.ds(h, h)], BF16)
        r2 = jnp.dot(x, pltpu.bitcast(wp[wi, pl.ds(h // 2, h // 2), :], BF16), preferred_element_type=F32)
        r = part[pi + z(), pl.ds(off, TM), :] + r2
        return r, slabs(r1) + slabs(r2)

    def b_proj(slot, sec, c):
        dst, off = ((q_s, 0), (k_s, HALO), (v_s, HALO))[sec]
        r, toks = mm2(xu, slot, sec * 8 + c, dst, c, off)
        dst[c, pl.ds(off, TM), :] = r
        return toks

    cexp = (DH ** -0.5) * math.log2(math.e)
    neg = -1e9 / (DH ** -0.5)
    flip = lane ^ 1

    def soft_units(t, rg):
        r0 = rg * 8
        st = {'ls': []}

        def logits(ws):
            zi = z()
            q = [q_s[zi + c, pl.ds(r0, 8), :] for c in range(8)]
            for w in ws:
                acc = q[0] * k_s[zi, pl.ds(HALO + r0 - DIL * w, 8), :]
                for c in range(1, 8):
                    acc = acc + q[c] * k_s[zi + c, pl.ds(HALO + r0 - DIL * w, 8), :]
                acc = acc + pltpu.roll(acc, 64, 1)
                acc = acc + jnp.take_along_axis(acc, flip, axis=1)
                if r0 - DIL * w < 0 and not (isinstance(t, int) and t > 0):
                    acc = jnp.where(row + (t * TM + r0 - DIL * w) >= 0, acc, neg)
                st['ls'].append(acc)
            if len(st['ls']) == WIN:
                ls = st['ls']
                m = functools.reduce(jnp.maximum, ls)
                ps = [jnp.exp2((l - m) * cexp) for l in ls]
                inv_den = 1.0 / tsum(ps)
                for w in range(WIN):
                    p_s[w, pl.ds(r0, 8), :] = ps[w] * inv_den
        return [('soft', 68, P(logits, range(0, 4))), ('soft', 108, P(logits, range(4, 8)))]

    def av_units(c, dyn=True):
        def av(rbs):
            for rb in rbs:
                r0 = rb * 16
                zi = z()
                cv = zi + c if dyn else c
                acc = p_s[zi, pl.ds(r0, 16), :] * v_s[cv, pl.ds(HALO + r0, 16), :]
                for w in range(1, WIN):
                    acc = acc + p_s[zi + w, pl.ds(r0, 16), :] * v_s[cv, pl.ds(HALO + r0 - DIL * w, 16), :]
                o_s[c, pl.ds(r0, 16), :] = acc.astype(BF16)
            if rbs[-1] == TM // 16 - 1:
                ou[0, :, pl.ds(c * 128, 128)] = pltpu.bitcast(o_s[c + z()], U32)
        return [('av', 64, P(av, (rb, rb + 1))) for rb in range(0, TM // 16, 2)]

    def b_out(t, c):
        r, toks = mm2(ou, 0, 24 + c, acc_s, c % 2, 0)
        ob_v[t, :, pl.ds(c * 128, 128)] = r.astype(BF16)
        return toks

    def gate(kind, tok):
        if kind == 'conv':
            ug_s[6 * 16 * NB + zero] = tok
        elif kind == 'soft':
            q_s[8 + zero, pl.ds(0, 8), :] = tok
        elif kind == 'av':
            p_s[8 + zero, pl.ds(0, 8), :] = tok
        elif kind == 'wv':
            w_v[32 + zero, pl.ds(0, 16), :] = pltpu.bitcast(tok, BF16)
        elif kind == 'wta':
            wt_a[8 + zero, pl.ds(0, 8), :] = pltpu.bitcast(tok, U32)
        elif kind == 'wtb':
            wt_b[8 + zero, pl.ds(0, 8), :] = pltpu.bitcast(tok, U32)
        elif kind == 'prep':
            kf_s[pl.ds(pl.multiple_of(S + 8 + zero * 8, 8), 8), :] = tok

    def a_consts(t):
        cs = pl.ds(al(t, CH), CH)
        skt_all = sk_ref[:, cs].astype(F32)
        return [skt_all[d:d + 1, :] for d in range(KS)], sd_ref[:, cs].astype(F32)

    def halo(ref):
        ref[:, pl.ds(0, HALO), :] = ref[:, pl.ds(TM, HALO), :]

    def pace(toks, units, lead=0):
        total = sum(u[1] for u in units)
        done = 0
        last = {}
        for kind, cost, fn in units:
            i = (len(toks) + lead) * done // total - lead
            if i >= 0 and last.get(kind) != i:
                gate(kind, toks[i])
                last[kind] = i
            fn()
            done += cost

    def merge(*lists):
        items = []
        for l in lists:
            if not l:
                continue
            tot = sum(u[1] for u in l)
            acc = 0
            for u in l:
                items.append((acc / tot, len(items), u))
                acc += u[1]
        return [u for _, _, u in sorted(items, key=lambda x: x[:2])]

    def emit(units):
        for u in units:
            u[2]()

    def tiny(i):
        return pltpu.make_async_copy(w_hbm.at[pl.ds(0, 16), pl.ds(0, 128)], tiny_v.at[i], sem_w.at[32 + i])

    nstart = [0]

    def start(ws, ins):
        for t, n in ins:
            in_copy(t, n).start()
        for sec in ws:
            for n in range(8):
                (w_copy(sec * 8 + n) if sec < 3 else wo_copy(n)).start()
        tiny(nstart[0]).wait()
        nstart[0] += 1

    def w_wait(sec):
        with jax.named_scope('w%d' % sec):
            for n in range(8):
                (w_copy(sec * 8 + n) if sec < 3 else wo_copy(n)).wait()

    def in_wait(*tn):
        with jax.named_scope('wI'):
            for t, n in tn:
                in_copy(t, n).wait()

    def soft_rows(t, a, b):
        return [u for rg in range(a, b) for u in soft_units(t, rg)]

    def prep_pair(t, c, skt):
        return prep_units(t, 2 * c, skt) + prep_units(t, 2 * c + 1, skt)

    def dft_pair(t, c, sd):
        toks = a_inv(t, 2 * c)
        a_inv(t, 2 * c + 1)
        toks += a_fwd(t + 1, 2 * c, sd)
        a_fwd(t + 1, 2 * c + 1, sd)
        return toks

    def tail_phases(t, extra, hook=None):
        halo(k_s)
        conv = [u for g in range(16) for u in conv_units(g)]
        ctot = sum(u[1] for u in conv)
        cdone = 0
        cw = CONV_W1 if extra else CONV_W
        for k in range(24):
            ph, c = divmod(k, 8)
            if hook is not None and k == 8:
                hook()
            toks = b_out(t, c) if ph == 2 else b_proj((t + 1) % 2, 1 - ph, c)
            mine = []
            while conv and cdone < ctot * sum(cw[:k + 1]) / sum(cw):
                cdone += conv[0][1]
                mine.append(conv.pop(0))
            units = merge(mine, av_units(c) if ph == 0 else [], extra.get(k, []))
            if units:
                pace(toks[:TAIL] if k == 23 else toks, units)
        copy_a(t).start()
        copy_b(t).start()

    for n in range(3):
        in_copy(0, n).start()
    for i in range(NTINY):
        tiny(i).start()
    k_s[:, pl.ds(0, HALO), :] = jnp.zeros((8, HALO, 128), F32)
    v_s[:, pl.ds(0, HALO), :] = jnp.zeros((8, HALO, 128), F32)
    kf_s[pl.ds(0, 8), :] = jnp.zeros((8, 128), F32)
    in_wait((0, 0), (0, 1), (0, 2))
    start([1], [(0, 3)])
    skt, sd = a_consts(0)
    emit(prep_pair(0, 0, skt))
    for c in range(8):
        toks = a_fwd(0, 2 * c, sd)
        a_fwd(0, 2 * c + 1, sd)
        if c < 7:
            pace(toks[:12], prep_pair(0, c + 1, skt), 4)
    conv = [conv_units(g) for g in range(16)]
    for g in range(PRO_CONV):
        if g == PRO_WQ:
            start([0], [])
        emit(conv[g])
    w_wait(1)
    in_wait((0, 3))
    stage_x(0, 0)
    emit(sel_units(1))
    emit(lane_units(1, 0))
    rest = conv[PRO_CONV:]
    for sec, nxt in ((1, 0), (0, 2)):
        for c in range(8):
            if c == 2:
                if sec == 1:
                    start([2], [])
                else:
                    start([], [(0, 4), (1, 0), (1, 1), (1, 2), (1, 3)])
            if c == 5:
                w_wait(nxt)
                sel = sel_units(nxt)
            toks = b_proj(0, sec, c)
            if c < 5:
                pace(toks, merge(lane_units(sec, c + 1), rest.pop(0) if rest else []))
            elif c < 7:
                pace(toks, merge(lane_units(sec, c + 1), sel[(c - 5) * 32:(c - 4) * 32]))
            else:
                pace(toks[:16], lane_units(nxt, 0))
    assert not rest
    for c in range(4):
        toks = b_proj(0, 2, c)
        pace(toks[:24] if c == 3 else toks,
             merge(lane_units(2, c + 1), soft_rows(0, (0, 5, 10, 15)[c], (5, 10, 15, 18)[c])))
    in_wait((0, 4), (1, 0), (1, 1), (1, 2), (1, 3))
    start([3], [])
    stage_x(1, 1)
    skt, sd = a_consts(1)
    emit(prep_pair(1, 0, skt))
    for c in range(4, 8):
        d = 2 * (c - 4)
        toks = b_proj(0, 2, c)
        pace(toks, merge(lane_units(2, c + 1) if c < 7 else [], soft_rows(0, 4 * c + 2, 4 * c + 4),
                         prep_pair(1, d + 1, skt)))
        toks = dft_pair(0, d, sd) + dft_pair(0, d + 1, sd)
        if c < 7:
            pace(toks, merge(soft_rows(0, 4 * c + 4, 4 * c + 6), prep_pair(1, d + 2, skt)))

    def hook():
        w_wait(3)
        start([], [(1, 4), (2, 0), (2, 1), (2, 2), (2, 3)])
    tail_phases(0, {8 + c: wo_units(c) for c in range(8)}, hook)

    assert nstart[0] == NTINY

    def loop(t, carry):
        in_copy(t + 1, 4).start()

        @pl.when(t + 2 < NSTEP)
        def _():
            for n in range(4):
                in_copy(t + 2, n).start()

        in_wait((t, 4), (t + 1, 0), (t + 1, 1), (t + 1, 2), (t + 1, 3))

        halo(v_s)
        skt, sd = a_consts(t + 1)
        stage_x(t + 1, (t + 1) % 2)
        emit(prep_pair(t + 1, 0, skt))
        for c in range(8):
            toks = b_proj(t % 2, 2, c) + dft_pair(t, c, sd)
            soft = soft_rows(1, 4 * c, 4 * c + 4)
            if c < 7:
                pace(toks, merge(soft, prep_pair(t + 1, c + 1, skt)), LEAD if c == 0 else 0)
            else:
                pace(toks[:FIN], soft)
        tail_phases(t, {})
        return carry
    jax.lax.fori_loop(1, NSTEP - 1, loop, 0)

    t = NSTEP - 1
    in_wait((t, 4))
    halo(v_s)
    for c in range(8):
        toks = b_proj(t % 2, 2, c)
        if c < 5:
            pace(toks, [u for rg in range(32) if rg * 5 // 32 == c for u in soft_units(t, rg)],
                 LEAD if c == 0 else 0)
        else:
            pace(toks, [u for cc in ((0, 1), (2, 3), (4, 5))[c - 5] for u in av_units(cc, False)])
    toks = []
    for i in range(NB):
        tk = a_inv(t, i)
        if i % 2 == 0:
            toks += tk
    pace(toks[:40], av_units(6, False) + av_units(7, False))
    copy_a(t).start()
    for c in range(8):
        b_out(t, c)
        if c % 2 == 1:
            copy_b_last(c // 2).start()
    with jax.named_scope('wOut'):
        for s in range(NSTEP - 1):
            copy_a(s).wait()
            copy_b(s).wait()
        copy_a(t).wait()
        for n in range(4):
            copy_b_last(n).wait()


@jax.jit
def pallas_concat_heads__ssm_conv_h3__sliding_local_dilated__prompt_kernel(
    A_q, A_k, A_v, A_shift_k, A_ssm_k, A_ssm_D, B_x, B_wqkv, B_wo,
):
    fwd, inv = _dft_consts()
    fwd = jnp.asarray(_pack_rows(fwd))
    inv = jnp.asarray(_pack_rows(inv))
    hbm = pl.BlockSpec(memory_space=pl.ANY)
    vmem = pl.BlockSpec(memory_space=pltpu.VMEM)
    smem = pl.BlockSpec(memory_space=pltpu.SMEM)
    out = pl.pallas_call(
        _kernel,
        in_specs=[smem, hbm, hbm, hbm, vmem, hbm, vmem, hbm, hbm, hbm, vmem, vmem],
        out_specs=hbm,
        out_shape=jax.ShapeDtypeStruct((S, 2 * D), BF16),
        scratch_shapes=[
            pltpu.VMEM((NSTEP, S, CH), BF16),
            pltpu.VMEM((NSTEP, S, CH), BF16),
            pltpu.VMEM((NSTEP, S, CH), BF16),
            pltpu.VMEM((NSTEP, CH, S), BF16),
            pltpu.VMEM((NSTEP, TM, D), BF16),
            pltpu.VMEM((33, D, 128), BF16),
            pltpu.VMEM((32, D // 2, 128), U32),
            pltpu.VMEM((9, D // 2, 128), U32),
            pltpu.VMEM((9, D // 2, 128), U32),
            pltpu.VMEM((2, TM // 2, D), U32),
            pltpu.VMEM((1, TM // 2, D), U32),
            pltpu.VMEM((2, TM, 128), F32),
            pltpu.VMEM((9, TM, 128), F32),
            pltpu.VMEM((8, TM + HALO, 128), F32),
            pltpu.VMEM((8, TM + HALO, 128), F32),
            pltpu.VMEM((WIN + 1, TM, 128), F32),
            pltpu.VMEM((8, TM, 128), BF16),
            pltpu.VMEM((S + 16, 128), F32),
            pltpu.VMEM((S, 128), BF16),
            pltpu.VMEM((6 * 16 * NB + 1, 8, 128), F32),
            pltpu.VMEM((NB, 2 * BL, 128), BF16),
            pltpu.VMEM((NSTEP, S, CH), BF16),
            pltpu.VMEM((NSTEP, TM, D), BF16),
            pltpu.VMEM((NTINY, 16, 128), BF16),
            pltpu.SemaphoreType.DMA((NSTEP, 5)),
            pltpu.SemaphoreType.DMA((32 + NTINY,)),
            pltpu.SemaphoreType.DMA((NSTEP, 5)),
        ],
        compiler_params=pltpu.CompilerParams(vmem_limit_bytes=100 * 1024 * 1024),
    )(jnp.zeros((NZ,), jnp.int32), A_q.reshape(S, D), A_k.reshape(S, D), A_v.reshape(S, D),
      A_shift_k.T, A_ssm_k, A_ssm_D.reshape(1, D),
      B_x.reshape(S, D), B_wqkv, B_wo, fwd, inv)
    return out.reshape(1, S, 2 * D)
```

```python
import functools
import math

import jax
import jax.numpy as jnp
import numpy as np
import jax.experimental.pallas as pl
import jax.experimental.pallas.tpu as pltpu

S = 2048
D = 1024
DH = 32
WIN = 8
DIL = 2
KS = 4
BL = 128
NB = S // BL
NSTEP = 8
TM = S // NSTEP
CH = D // NSTEP
HALO = 16
F32 = jnp.float32
BF16 = jnp.bfloat16
U32 = jnp.uint32


def _dft_consts():
    n = 2 * BL
    fwd = np.zeros((n, BL), np.float64)
    inv = np.zeros((BL, n), np.float64)
    t = np.arange(BL)
    for g in range(16):
        for r in range(8):
            f = 2 * (8 * g + r)
            ang = 2.0 * np.pi * (f + 0.5) * t / n
            fwd[16 * g + r] = np.cos(ang)
            fwd[16 * g + 8 + r] = -np.sin(ang)
            inv[:, 16 * g + r] = np.cos(ang) * (2.0 / n)
            inv[:, 16 * g + 8 + r] = -np.sin(ang) * (2.0 / n)
    return fwd.astype(np.float32), inv.astype(np.float32)


NZ = 64
NTINY = 6
LEAD = 8
FIN = 44
TAIL = 12
CONV_W = [3] * 8 + [8] * 15 + [3]
CONV_W1 = [4] * 8 + [6] * 8 + [9] * 7 + [3]
PRO_CONV = 12
PRO_WQ = 8


def _pack_rows(a):
    b = np.asarray(a, dtype=jnp.bfloat16).view(np.uint16).astype(np.uint32)
    return (b[0::2] | (b[1::2] << 16))[None]


def _kernel(zero_ref, aq_hbm, ak_hbm, av_hbm, sk_ref, hk_hbm, sd_ref, x_hbm, w_hbm, wo_hbm,
            fwd_ref, inv_ref, out_hbm,
            aq_v, ak_v, av_v, hk_v, x_v, w_v, wp, wt_a, wt_b,
            xu, ou, acc_s, q_s, k_s, v_s, p_s, o_s, kf_s, kv_s, ug_s, y_s, oa_v, ob_v, tiny_v,
            sem_in, sem_w, sem_out):
    lane = jax.lax.broadcasted_iota(jnp.int32, (8, 128), 1)
    row = jax.lax.broadcasted_iota(jnp.int32, (8, 128), 0)
    zero = zero_ref[0]
    zcount = [0]
    P = functools.partial

    def z():
        zcount[0] = zcount[0] % (NZ - 1) + 1
        return zero_ref[zcount[0]]

    def al(i, m):
        return i * m if isinstance(i, int) else pl.multiple_of(i * m, m)

    def in_copy(t, n):
        cs = pl.ds(al(t, CH), CH)
        rs = pl.ds(al(t, TM), TM)
        if n == 0:
            src, dst = ak_hbm.at[:, cs], ak_v
        elif n == 1:
            src, dst = av_hbm.at[:, cs], av_v
        elif n == 2:
            src, dst = hk_hbm.at[cs, :], hk_v
        elif n == 3:
            src, dst = x_hbm.at[rs, :], x_v
        else:
            src, dst = aq_hbm.at[:, cs], aq_v
        return pltpu.make_async_copy(src, dst.at[t], sem_in.at[t, n])

    def w_copy(n):
        return pltpu.make_async_copy(w_hbm.at[:, pl.ds(n * 128, 128)], w_v.at[n], sem_w.at[n])

    def wo_copy(n):
        return pltpu.make_async_copy(wo_hbm.at[:, pl.ds(n * 128, 128)], w_v.at[24 + n], sem_w.at[24 + n])

    def copy_a(t):
        return pltpu.make_async_copy(oa_v.at[t], out_hbm.at[:, pl.ds(al(t, CH), CH)], sem_out.at[t, 0])

    def copy_b(t):
        return pltpu.make_async_copy(
            ob_v.at[t], out_hbm.at[pl.ds(al(t, TM), TM), pl.ds(D, D)], sem_out.at[t, 1])

    def copy_b_last(n):
        t = NSTEP - 1
        return pltpu.make_async_copy(
            ob_v.at[t, :, pl.ds(n * 256, 256)],
            out_hbm.at[pl.ds(t * TM, TM), pl.ds(D + n * 256, 256)], sem_out.at[t, 1 + n])

    def xor_select(c, sel):
        for s in range(3):
            bit = (sel & (1 << s)) != 0
            c = [jnp.where(bit, c[i ^ (1 << s)], c[i]) for i in range(8)]
        return c

    def tsum(vals):
        return functools.reduce(lambda a, b: a + b, vals)

    def lane_src(j):
        return (((lane >> 4) & 3) << 5) | ((lane >> 6) << 4) | ((((lane >> 1) & 7) ^ j) << 1) | (lane & 1)

    def wtmp(sec):
        return (wt_b, wt_a, wt_a)[sec], ('wtb', 'wta', 'wta')[sec]

    def sel_units(sec):
        wt, _ = wtmp(sec)

        def sel(rb):
            c = [pltpu.bitcast(w_v[sec * 8 + i, pl.ds(rb * 16, 16), :], U32) for i in range(8)]
            c = xor_select(c, lane >> 1)
            for j in range(8):
                wt[j, pl.ds(rb * 8, 8), :] = c[j]
        return [('wv', 32, P(sel, rb)) for rb in range(64)]

    def lane_units(sec, j):
        wt, kind = wtmp(sec)

        def lanes(rb):
            zi = z()
            for r in range(rb * 64, rb * 64 + 64, 8):
                wp[sec * 8 + j, pl.ds(r, 8), :] = jnp.take_along_axis(
                    wt[zi + j, pl.ds(r, 8), :], lane_src(j), axis=1)
        return [(kind, 32, P(lanes, rb)) for rb in range(8)]

    def wo_units(c):
        def rows(mp):
            m = ((mp & 3) << 1) | (mp >> 2)
            tr = [pltpu.bitcast(w_v[24 + c, pl.ds(r * 128 + m * 16, 16), :], U32) for r in range(8)]
            tr = xor_select(tr, row)
            for j in range(8):
                wp[24 + c, pl.ds(j * 64 + mp * 8, 8), :] = (
                    jnp.take_along_axis(tr[j], row ^ j, axis=0) if j else tr[j])
        return [('wv', 40, P(rows, mp)) for mp in range(8)]

    def a_prep(t, r0, n, skt):
        kf_s[pl.ds(8 + r0, n), :] = ak_v[t, pl.ds(r0, n), :].astype(F32)
        ksh = kf_s[pl.ds(8 + r0, n), :] * skt[0]
        for d in range(1, KS):
            ksh = ksh + kf_s[pl.ds(8 + r0 - d, n), :] * skt[d]
        kv_s[pl.ds(r0, n), :] = (ksh * av_v[t, pl.ds(r0, n), :].astype(F32)).astype(BF16)

    def prep_units(t, j, skt):
        return [('prep', 48, P(a_prep, t, j * BL + r, 32, skt)) for r in range(0, BL, 32)]

    def slabs(r):
        return [r[i:i + 8] for i in range(0, r.shape[0], 16)]

    def ug(plane, g, j):
        return (plane * 16 + g) * NB + j

    def a_fwd(t, j, sd):
        fwd = pltpu.bitcast(fwd_ref[z()], BF16)
        u = jnp.dot(fwd, kv_s[pl.ds(j * BL, BL), :], preferred_element_type=F32)
        fwd = pltpu.bitcast(fwd_ref[z()], BF16)
        h = jax.lax.dot_general(fwd, hk_v[t, :, pl.ds(j * BL, BL)],
                                (((1,), (1,)), ((), ())), preferred_element_type=F32)
        for g in range(16):
            ur, ui = u[16 * g:16 * g + 8], u[16 * g + 8:16 * g + 16]
            ug_s[ug(0, g, j)] = ur + ui
            ug_s[ug(1, g, j)] = ur
            ug_s[ug(2, g, j)] = ui
            hr, hi = h[16 * g:16 * g + 8], h[16 * g + 8:16 * g + 16]
            if j == 0:
                hr = hr + sd
            ug_s[ug(3, g, j)] = hr
            ug_s[ug(4, g, j)] = hi - hr
            ug_s[ug(5, g, j)] = hr + hi
        return slabs(u)

    def conv_units(g):
        st = {'prev': None}

        def toep(ib, pl_):
            zi = z()
            acc = [None] * 4 if pl_ == 0 else list(st[0])
            gs = {}
            for jb in range(ib + 1):
                us = [ug_s[zi + ug(pl_, g, 4 * jb + b)] for b in range(4)]
                m0 = 4 * (ib - jb)
                gs = {m: gs[m] if m in gs else ug_s[zi + ug(3 + pl_, g, m)]
                      for m in range(max(m0 - 3, 0), m0 + 4)}
                for a in range(4):
                    for b in range(4):
                        m = m0 + a - b
                        if m < 0:
                            continue
                        pr = us[b] * gs[m]
                        if acc[a] is None:
                            acc[a] = pr
                        else:
                            acc[a] = acc[a] + pr if pl_ < 2 else acc[a] - pr
            st[pl_] = acc
            if pl_ == 2:
                im, re = st[1], st[2]
                for a in range(4):
                    prev = st['prev']
                    if prev is None:
                        yr, yi = re[a], im[a]
                    else:
                        yr, yi = re[a] - prev[1], im[a] + prev[0]
                    st['prev'] = (re[a], im[a])
                    y_s[4 * ib + a, pl.ds(16 * g, 16), :] = jnp.concatenate([yr, yi], axis=0).astype(BF16)
        return [('conv', 20 + 32 * ib + (12 if pl_ == 2 else 0), P(toep, ib, pl_))
                for ib in range(4) for pl_ in range(3)]

    def a_conv(g):
        for _, _, fn in conv_units(g):
            fn()

    def a_inv(t, i):
        rs = pl.ds(i * BL, BL)
        inv = pltpu.bitcast(inv_ref[z()], BF16)
        y = jnp.dot(inv, y_s[i], preferred_element_type=F32)
        r = aq_v[t, rs, :].astype(F32) * y
        oa_v[t, rs, :] = r.astype(BF16)
        return slabs(y)

    def stage_x(t, slot):
        xu[slot] = pltpu.bitcast(x_v[t], U32)

    def mm2(lhs, li, wi, part, pi, off):
        h = D // 2
        x = pltpu.bitcast(lhs[li + z(), :, pl.ds(0, h)], BF16)
        r1 = jnp.dot(x, pltpu.bitcast(wp[wi, pl.ds(0, h // 2), :], BF16), preferred_element_type=F32)
        part[pi, pl.ds(off, TM), :] = r1
        x = pltpu.bitcast(lhs[li + z(), :, pl.ds(h, h)], BF16)
        r2 = jnp.dot(x, pltpu.bitcast(wp[wi, pl.ds(h // 2, h // 2), :], BF16), preferred_element_type=F32)
        r = part[pi + z(), pl.ds(off, TM), :] + r2
        return r, slabs(r1) + slabs(r2)

    def b_proj(slot, sec, c):
        dst, off = ((q_s, 0), (k_s, HALO), (v_s, HALO))[sec]
        r, toks = mm2(xu, slot, sec * 8 + c, dst, c, off)
        dst[c, pl.ds(off, TM), :] = r
        return toks

    cexp = (DH ** -0.5) * math.log2(math.e)
    neg = -1e9 / (DH ** -0.5)
    flip = lane ^ 1

    def soft_units(t, rg):
        r0 = rg * 8
        st = {'ls': []}

        def logits(ws):
            zi = z()
            q = [q_s[zi + c, pl.ds(r0, 8), :] for c in range(8)]
            for w in ws:
                acc = q[0] * k_s[zi, pl.ds(HALO + r0 - DIL * w, 8), :]
                for c in range(1, 8):
                    acc = acc + q[c] * k_s[zi + c, pl.ds(HALO + r0 - DIL * w, 8), :]
                acc = acc + pltpu.roll(acc, 64, 1)
                acc = acc + jnp.take_along_axis(acc, flip, axis=1)
                if r0 - DIL * w < 0 and not (isinstance(t, int) and t > 0):
                    acc = jnp.where(row + (t * TM + r0 - DIL * w) >= 0, acc, neg)
                st['ls'].append(acc)
            if len(st['ls']) == WIN:
                ls = st['ls']
                m = functools.reduce(jnp.maximum, ls)
                ps = [jnp.exp2((l - m) * cexp) for l in ls]
                inv_den = 1.0 / tsum(ps)
                for w in range(WIN):
                    p_s[w, pl.ds(r0, 8), :] = ps[w] * inv_den
        return [('soft', 68, P(logits, range(0, 4))), ('soft', 108, P(logits, range(4, 8)))]

    def av_units(c, dyn=True):
        def av(rbs):
            for rb in rbs:
                r0 = rb * 16
                zi = z()
                cv = zi + c if dyn else c
                acc = p_s[zi, pl.ds(r0, 16), :] * v_s[cv, pl.ds(HALO + r0, 16), :]
                for w in range(1, WIN):
                    acc = acc + p_s[zi + w, pl.ds(r0, 16), :] * v_s[cv, pl.ds(HALO + r0 - DIL * w, 16), :]
                o_s[c, pl.ds(r0, 16), :] = acc.astype(BF16)
            if rbs[-1] == TM // 16 - 1:
                ou[0, :, pl.ds(c * 128, 128)] = pltpu.bitcast(o_s[c + z()], U32)
        return [('av', 64, P(av, (rb, rb + 1))) for rb in range(0, TM // 16, 2)]

    def b_out(t, c):
        r, toks = mm2(ou, 0, 24 + c, acc_s, c % 2, 0)
        ob_v[t, :, pl.ds(c * 128, 128)] = r.astype(BF16)
        return toks

    def gate(kind, tok):
        if kind == 'conv':
            ug_s[6 * 16 * NB + zero] = tok
        elif kind == 'soft':
            q_s[8 + zero, pl.ds(0, 8), :] = tok
        elif kind == 'av':
            p_s[8 + zero, pl.ds(0, 8), :] = tok
        elif kind == 'wv':
            w_v[32 + zero, pl.ds(0, 16), :] = pltpu.bitcast(tok, BF16)
        elif kind == 'wta':
            wt_a[8 + zero, pl.ds(0, 8), :] = pltpu.bitcast(tok, U32)
        elif kind == 'wtb':
            wt_b[8 + zero, pl.ds(0, 8), :] = pltpu.bitcast(tok, U32)
        elif kind == 'prep':
            kf_s[pl.ds(pl.multiple_of(S + 8 + zero * 8, 8), 8), :] = tok

    def a_consts(t):
        cs = pl.ds(al(t, CH), CH)
        skt_all = sk_ref[:, cs].astype(F32)
        return [skt_all[d:d + 1, :] for d in range(KS)], sd_ref[:, cs].astype(F32)

    def halo(ref):
        ref[:, pl.ds(0, HALO), :] = ref[:, pl.ds(TM, HALO), :]

    def pace(toks, units, lead=0):
        total = sum(u[1] for u in units)
        done = 0
        last = {}
        for kind, cost, fn in units:
            i = (len(toks) + lead) * done // total - lead
            if i >= 0 and last.get(kind) != i:
                gate(kind, toks[i])
                last[kind] = i
            fn()
            done += cost

    def merge(*lists):
        items = []
        for l in lists:
            if not l:
                continue
            tot = sum(u[1] for u in l)
            acc = 0
            for u in l:
                items.append((acc / tot, len(items), u))
                acc += u[1]
        return [u for _, _, u in sorted(items, key=lambda x: x[:2])]

    def emit(units):
        for u in units:
            u[2]()

    def tiny(i):
        return pltpu.make_async_copy(w_hbm.at[pl.ds(0, 16), pl.ds(0, 128)], tiny_v.at[i], sem_w.at[32 + i])

    nstart = [0]

    def start(ws, ins):
        for t, n in ins:
            in_copy(t, n).start()
        for sec in ws:
            for n in range(8):
                (w_copy(sec * 8 + n) if sec < 3 else wo_copy(n)).start()
        tiny(nstart[0]).wait()
        nstart[0] += 1

    def w_wait(sec):
        for n in range(8):
            (w_copy(sec * 8 + n) if sec < 3 else wo_copy(n)).wait()

    def in_wait(*tn):
        for t, n in tn:
            in_copy(t, n).wait()

    def soft_rows(t, a, b):
        return [u for rg in range(a, b) for u in soft_units(t, rg)]

    def prep_pair(t, c, skt):
        return prep_units(t, 2 * c, skt) + prep_units(t, 2 * c + 1, skt)

    def dft_pair(t, c, sd):
        toks = a_inv(t, 2 * c)
        a_inv(t, 2 * c + 1)
        toks += a_fwd(t + 1, 2 * c, sd)
        a_fwd(t + 1, 2 * c + 1, sd)
        return toks

    def tail_phases(t, extra, hook=None):
        halo(k_s)
        conv = [u for g in range(16) for u in conv_units(g)]
        ctot = sum(u[1] for u in conv)
        cdone = 0
        cw = CONV_W1 if extra else CONV_W
        for k in range(24):
            ph, c = divmod(k, 8)
            if hook is not None and k == 8:
                hook()
            toks = b_out(t, c) if ph == 2 else b_proj((t + 1) % 2, 1 - ph, c)
            mine = []
            while conv and cdone < ctot * sum(cw[:k + 1]) / sum(cw):
                cdone += conv[0][1]
                mine.append(conv.pop(0))
            units = merge(mine, av_units(c) if ph == 0 else [], extra.get(k, []))
            if units:
                pace(toks[:TAIL] if k == 23 else toks, units)
        copy_a(t).start()
        copy_b(t).start()

    for n in range(3):
        in_copy(0, n).start()
    for i in range(NTINY):
        tiny(i).start()
    k_s[:, pl.ds(0, HALO), :] = jnp.zeros((8, HALO, 128), F32)
    v_s[:, pl.ds(0, HALO), :] = jnp.zeros((8, HALO, 128), F32)
    kf_s[pl.ds(0, 8), :] = jnp.zeros((8, 128), F32)
    in_wait((0, 0), (0, 1), (0, 2))
    start([1], [(0, 3)])
    skt, sd = a_consts(0)
    emit(prep_pair(0, 0, skt))
    for c in range(8):
        toks = a_fwd(0, 2 * c, sd)
        a_fwd(0, 2 * c + 1, sd)
        if c < 7:
            pace(toks[:12], prep_pair(0, c + 1, skt), 4)
    conv = [conv_units(g) for g in range(16)]
    for g in range(PRO_CONV):
        if g == PRO_WQ:
            start([0], [])
        emit(conv[g])
    w_wait(1)
    in_wait((0, 3))
    stage_x(0, 0)
    emit(sel_units(1))
    emit(lane_units(1, 0))
    rest = conv[PRO_CONV:]
    for sec, nxt in ((1, 0), (0, 2)):
        for c in range(8):
            if c == 2:
                if sec == 1:
                    start([2], [])
                else:
                    start([], [(0, 4), (1, 0), (1, 1), (1, 2), (1, 3)])
            if c == 5:
                w_wait(nxt)
                sel = sel_units(nxt)
            toks = b_proj(0, sec, c)
            if c < 5:
                pace(toks, merge(lane_units(sec, c + 1), rest.pop(0) if rest else []))
            elif c < 7:
                pace(toks, merge(lane_units(sec, c + 1), sel[(c - 5) * 32:(c - 4) * 32]))
            else:
                pace(toks[:16], lane_units(nxt, 0))
    assert not rest
    for c in range(4):
        toks = b_proj(0, 2, c)
        pace(toks[:24] if c == 3 else toks,
             merge(lane_units(2, c + 1), soft_rows(0, (0, 5, 10, 15)[c], (5, 10, 15, 18)[c])))
    in_wait((0, 4), (1, 0), (1, 1), (1, 2), (1, 3))
    start([3], [])
    stage_x(1, 1)
    skt, sd = a_consts(1)
    emit(prep_pair(1, 0, skt))
    for c in range(4, 8):
        d = 2 * (c - 4)
        toks = b_proj(0, 2, c)
        pace(toks, merge(lane_units(2, c + 1) if c < 7 else [], soft_rows(0, 4 * c + 2, 4 * c + 4),
                         prep_pair(1, d + 1, skt)))
        toks = dft_pair(0, d, sd) + dft_pair(0, d + 1, sd)
        if c < 7:
            pace(toks, merge(soft_rows(0, 4 * c + 4, 4 * c + 6), prep_pair(1, d + 2, skt)))

    def hook():
        w_wait(3)
        start([], [(1, 4), (2, 0), (2, 1), (2, 2), (2, 3)])
    tail_phases(0, {8 + c: wo_units(c) for c in range(8)}, hook)

    assert nstart[0] == NTINY

    def loop(t, carry):
        in_copy(t + 1, 4).start()

        @pl.when(t + 2 < NSTEP)
        def _():
            for n in range(4):
                in_copy(t + 2, n).start()

        in_wait((t, 4), (t + 1, 0), (t + 1, 1), (t + 1, 2), (t + 1, 3))

        halo(v_s)
        skt, sd = a_consts(t + 1)
        stage_x(t + 1, (t + 1) % 2)
        emit(prep_pair(t + 1, 0, skt))
        for c in range(8):
            toks = b_proj(t % 2, 2, c) + dft_pair(t, c, sd)
            soft = soft_rows(1, 4 * c, 4 * c + 4)
            if c < 7:
                pace(toks, merge(soft, prep_pair(t + 1, c + 1, skt)), LEAD if c == 0 else 0)
            else:
                pace(toks[:FIN], soft)
        tail_phases(t, {})
        return carry
    jax.lax.fori_loop(1, NSTEP - 1, loop, 0)

    t = NSTEP - 1
    in_wait((t, 4))
    halo(v_s)
    for c in range(8):
        toks = b_proj(t % 2, 2, c)
        if c < 5:
            pace(toks, [u for rg in range(32) if rg * 5 // 32 == c for u in soft_units(t, rg)],
                 LEAD if c == 0 else 0)
        else:
            pace(toks, [u for cc in ((0, 1), (2, 3), (4, 5))[c - 5] for u in av_units(cc, False)])
    toks = []
    for i in range(NB):
        tk = a_inv(t, i)
        if i % 2 == 0:
            toks += tk
    pace(toks[:40], av_units(6, False) + av_units(7, False))
    copy_a(t).start()
    for c in range(8):
        b_out(t, c)
        if c % 2 == 1:
            copy_b_last(c // 2).start()
    for s in range(NSTEP - 1):
        copy_a(s).wait()
        copy_b(s).wait()
    copy_a(t).wait()
    for n in range(4):
        copy_b_last(n).wait()


@jax.jit
def pallas_concat_heads__ssm_conv_h3__sliding_local_dilated__prompt_kernel(
    A_q, A_k, A_v, A_shift_k, A_ssm_k, A_ssm_D, B_x, B_wqkv, B_wo,
):
    fwd, inv = _dft_consts()
    fwd = jnp.asarray(_pack_rows(fwd))
    inv = jnp.asarray(_pack_rows(inv))
    hbm = pl.BlockSpec(memory_space=pl.ANY)
    vmem = pl.BlockSpec(memory_space=pltpu.VMEM)
    smem = pl.BlockSpec(memory_space=pltpu.SMEM)
    out = pl.pallas_call(
        _kernel,
        in_specs=[smem, hbm, hbm, hbm, vmem, hbm, vmem, hbm, hbm, hbm, vmem, vmem],
        out_specs=hbm,
        out_shape=jax.ShapeDtypeStruct((S, 2 * D), BF16),
        scratch_shapes=[
            pltpu.VMEM((NSTEP, S, CH), BF16),
            pltpu.VMEM((NSTEP, S, CH), BF16),
            pltpu.VMEM((NSTEP, S, CH), BF16),
            pltpu.VMEM((NSTEP, CH, S), BF16),
            pltpu.VMEM((NSTEP, TM, D), BF16),
            pltpu.VMEM((33, D, 128), BF16),
            pltpu.VMEM((32, D // 2, 128), U32),
            pltpu.VMEM((9, D // 2, 128), U32),
            pltpu.VMEM((9, D // 2, 128), U32),
            pltpu.VMEM((2, TM // 2, D), U32),
            pltpu.VMEM((1, TM // 2, D), U32),
            pltpu.VMEM((2, TM, 128), F32),
            pltpu.VMEM((9, TM, 128), F32),
            pltpu.VMEM((8, TM + HALO, 128), F32),
            pltpu.VMEM((8, TM + HALO, 128), F32),
            pltpu.VMEM((WIN + 1, TM, 128), F32),
            pltpu.VMEM((8, TM, 128), BF16),
            pltpu.VMEM((S + 16, 128), F32),
            pltpu.VMEM((S, 128), BF16),
            pltpu.VMEM((6 * 16 * NB + 1, 8, 128), F32),
            pltpu.VMEM((NB, 2 * BL, 128), BF16),
            pltpu.VMEM((NSTEP, S, CH), BF16),
            pltpu.VMEM((NSTEP, TM, D), BF16),
            pltpu.VMEM((NTINY, 16, 128), BF16),
            pltpu.SemaphoreType.DMA((NSTEP, 5)),
            pltpu.SemaphoreType.DMA((32 + NTINY,)),
            pltpu.SemaphoreType.DMA((NSTEP, 5)),
        ],
        compiler_params=pltpu.CompilerParams(vmem_limit_bytes=100 * 1024 * 1024),
    )(jnp.zeros((NZ,), jnp.int32), A_q.reshape(S, D), A_k.reshape(S, D), A_v.reshape(S, D),
      A_shift_k.T, A_ssm_k, A_ssm_D.reshape(1, D),
      B_x.reshape(S, D), B_wqkv, B_wo, fwd, inv)
    return out.reshape(1, S, 2 * D)
```

```python
import functools
import math

import jax
import jax.numpy as jnp
import numpy as np
import jax.experimental.pallas as pl
import jax.experimental.pallas.tpu as pltpu

S = 2048
D = 1024
DH = 32
WIN = 8
DIL = 2
KS = 4
BL = 128
NB = S // BL
NSTEP = 8
TM = S // NSTEP
CH = D // NSTEP
HALO = 16
F32 = jnp.float32
BF16 = jnp.bfloat16
U32 = jnp.uint32


def _dft_consts():
    n = 2 * BL
    fwd = np.zeros((n, BL), np.float64)
    inv = np.zeros((BL, n), np.float64)
    t = np.arange(BL)
    for g in range(16):
        for r in range(8):
            f = 2 * (8 * g + r)
            ang = 2.0 * np.pi * (f + 0.5) * t / n
            fwd[16 * g + r] = np.cos(ang)
            fwd[16 * g + 8 + r] = -np.sin(ang)
            inv[:, 16 * g + r] = np.cos(ang) * (2.0 / n)
            inv[:, 16 * g + 8 + r] = -np.sin(ang) * (2.0 / n)
    return fwd.astype(np.float32), inv.astype(np.float32)


NZ = 64
NTINY = 3
NH = 2
LEAD = 8
FIN = 44
TAIL = 12
CONV_W = [3] * 8 + [8] * 15 + [3]
CONV_W1 = [4] * 8 + [6] * 8 + [9] * 7 + [3]
PRO_G = (7, 9, 11, 13, 16)
PRO_SOFT = 30


def _pack_rows(a):
    b = np.asarray(a, dtype=jnp.bfloat16).view(np.uint16).astype(np.uint32)
    return (b[0::2] | (b[1::2] << 16))[None]


def _kernel(zero_ref, aq_hbm, ak_hbm, av_hbm, sk_ref, hk_hbm, sd_ref, x_hbm, w_hbm, wo_hbm,
            fwd_ref, inv_ref, out_hbm,
            aq_v, ak_v, av_v, hk_v, x_v, w_v, wp, wt_a, wt_b,
            xu, ou, acc_s, q_s, k_s, v_s, p_s, o_s, kf_s, kv_s, ug_s, y_s, oa_v, ob_v, tiny_v, k0_s,
            sem_in, sem_w, sem_out, sem_h, sem_k):
    lane = jax.lax.broadcasted_iota(jnp.int32, (8, 128), 1)
    row = jax.lax.broadcasted_iota(jnp.int32, (8, 128), 0)
    zero = zero_ref[0]
    zcount = [0]
    P = functools.partial

    def z():
        zcount[0] = zcount[0] % (NZ - 1) + 1
        return zero_ref[zcount[0]]

    def al(i, m):
        return i * m if isinstance(i, int) else pl.multiple_of(i * m, m)

    def in_copy(t, n):
        cs = pl.ds(al(t, CH), CH)
        rs = pl.ds(al(t, TM), TM)
        if n == 0:
            src, dst = ak_hbm.at[:, cs], ak_v
        elif n == 1:
            src, dst = av_hbm.at[:, cs], av_v
        elif n == 2:
            src, dst = hk_hbm.at[cs, :], hk_v
        elif n == 3:
            src, dst = x_hbm.at[rs, :], x_v
        else:
            src, dst = aq_hbm.at[:, cs], aq_v
        return pltpu.make_async_copy(src, dst.at[t], sem_in.at[t, n])

    def first_copy(h, n):
        ts = pl.ds(h * (S // NH), S // NH)
        cs = pl.ds(0, CH)
        if n == 2:
            src, dst = hk_hbm.at[cs, ts], hk_v.at[0, :, ts]
        else:
            src, dst = (ak_hbm, av_hbm)[n].at[ts, cs], (ak_v, av_v)[n].at[0, ts, :]
        return pltpu.make_async_copy(src, dst, sem_h.at[h, n])

    def wh_copy(p, n):
        col = (8, 0, 16)[p // 2] + n
        rs = pl.ds((p % 2) * (D // 2), D // 2)
        return pltpu.make_async_copy(w_hbm.at[rs, pl.ds(col * 128, 128)], w_v.at[col, rs, :],
                                     sem_k.at[p, n])

    def wo_copy(n):
        return pltpu.make_async_copy(wo_hbm.at[:, pl.ds(n * 128, 128)], w_v.at[24 + n], sem_w.at[24 + n])

    def copy_a(t):
        return pltpu.make_async_copy(oa_v.at[t], out_hbm.at[:, pl.ds(al(t, CH), CH)], sem_out.at[t, 0])

    def copy_b(t):
        return pltpu.make_async_copy(
            ob_v.at[t], out_hbm.at[pl.ds(al(t, TM), TM), pl.ds(D, D)], sem_out.at[t, 1])

    def copy_b_last(n):
        t = NSTEP - 1
        return pltpu.make_async_copy(
            ob_v.at[t, :, pl.ds(n * 256, 256)],
            out_hbm.at[pl.ds(t * TM, TM), pl.ds(D + n * 256, 256)], sem_out.at[t, 1 + n])

    def xor_select(c, sel):
        for s in range(3):
            bit = (sel & (1 << s)) != 0
            c = [jnp.where(bit, c[i ^ (1 << s)], c[i]) for i in range(8)]
        return c

    def tsum(vals):
        return functools.reduce(lambda a, b: a + b, vals)

    def lane_src(j):
        return (((lane >> 4) & 3) << 5) | ((lane >> 6) << 4) | ((((lane >> 1) & 7) ^ j) << 1) | (lane & 1)

    def wtmp(sec):
        return (wt_b, wt_a, wt_a)[sec], ('wtb', 'wta', 'wta')[sec]

    def sel_units(sec):
        wt, _ = wtmp(sec)

        def sel(rb):
            c = [pltpu.bitcast(w_v[sec * 8 + i, pl.ds(rb * 16, 16), :], U32) for i in range(8)]
            c = xor_select(c, lane >> 1)
            for j in range(8):
                wt[j, pl.ds(rb * 8, 8), :] = c[j]
        return [('wv', 32, P(sel, rb)) for rb in range(64)]

    def lane_units(sec, j):
        wt, kind = wtmp(sec)

        def lanes(rb):
            zi = z()
            for r in range(rb * 64, rb * 64 + 64, 8):
                wp[sec * 8 + j, pl.ds(r, 8), :] = jnp.take_along_axis(
                    wt[zi + j, pl.ds(r, 8), :], lane_src(j), axis=1)
        return [(kind, 32, P(lanes, rb)) for rb in range(8)]

    def wo_units(c):
        def rows(mp):
            m = ((mp & 3) << 1) | (mp >> 2)
            tr = [pltpu.bitcast(w_v[24 + c, pl.ds(r * 128 + m * 16, 16), :], U32) for r in range(8)]
            tr = xor_select(tr, row)
            for j in range(8):
                wp[24 + c, pl.ds(j * 64 + mp * 8, 8), :] = (
                    jnp.take_along_axis(tr[j], row ^ j, axis=0) if j else tr[j])
        return [('wv', 40, P(rows, mp)) for mp in range(8)]

    def a_prep(t, r0, n, skt):
        kf_s[pl.ds(8 + r0, n), :] = ak_v[t, pl.ds(r0, n), :].astype(F32)
        ksh = kf_s[pl.ds(8 + r0, n), :] * skt[0]
        for d in range(1, KS):
            ksh = ksh + kf_s[pl.ds(8 + r0 - d, n), :] * skt[d]
        kv_s[pl.ds(r0, n), :] = (ksh * av_v[t, pl.ds(r0, n), :].astype(F32)).astype(BF16)

    def prep_units(t, j, skt):
        return [('prep', 48, P(a_prep, t, j * BL + r, 32, skt)) for r in range(0, BL, 32)]

    def slabs(r):
        return [r[i:i + 8] for i in range(0, r.shape[0], 16)]

    def ug(plane, g, j):
        return (plane * 16 + g) * NB + j

    def a_fwd(t, j, sd):
        fwd = pltpu.bitcast(fwd_ref[z()], BF16)
        u = jnp.dot(fwd, kv_s[pl.ds(j * BL, BL), :], preferred_element_type=F32)
        fwd = pltpu.bitcast(fwd_ref[z()], BF16)
        h = jax.lax.dot_general(fwd, hk_v[t, :, pl.ds(j * BL, BL)],
                                (((1,), (1,)), ((), ())), preferred_element_type=F32)
        for g in range(16):
            ur, ui = u[16 * g:16 * g + 8], u[16 * g + 8:16 * g + 16]
            ug_s[ug(0, g, j)] = ur + ui
            ug_s[ug(1, g, j)] = ur
            ug_s[ug(2, g, j)] = ui
            hr, hi = h[16 * g:16 * g + 8], h[16 * g + 8:16 * g + 16]
            if j == 0:
                hr = hr + sd
            ug_s[ug(3, g, j)] = hr
            ug_s[ug(4, g, j)] = hi - hr
            ug_s[ug(5, g, j)] = hr + hi
        return slabs(u)

    def conv_units(g):
        st = {'prev': None}

        def toep(ib, pl_):
            zi = z()
            acc = [None] * 4 if pl_ == 0 else list(st[0])
            gs = {}
            for jb in range(ib + 1):
                us = [ug_s[zi + ug(pl_, g, 4 * jb + b)] for b in range(4)]
                m0 = 4 * (ib - jb)
                gs = {m: gs[m] if m in gs else ug_s[zi + ug(3 + pl_, g, m)]
                      for m in range(max(m0 - 3, 0), m0 + 4)}
                for a in range(4):
                    for b in range(4):
                        m = m0 + a - b
                        if m < 0:
                            continue
                        pr = us[b] * gs[m]
                        if acc[a] is None:
                            acc[a] = pr
                        else:
                            acc[a] = acc[a] + pr if pl_ < 2 else acc[a] - pr
            st[pl_] = acc
            if pl_ == 2:
                im, re = st[1], st[2]
                for a in range(4):
                    prev = st['prev']
                    if prev is None:
                        yr, yi = re[a], im[a]
                    else:
                        yr, yi = re[a] - prev[1], im[a] + prev[0]
                    st['prev'] = (re[a], im[a])
                    y_s[4 * ib + a, pl.ds(16 * g, 16), :] = jnp.concatenate([yr, yi], axis=0).astype(BF16)
        return [('conv', 20 + 32 * ib + (12 if pl_ == 2 else 0), P(toep, ib, pl_))
                for ib in range(4) for pl_ in range(3)]

    def a_conv(g):
        for _, _, fn in conv_units(g):
            fn()

    def a_inv(t, i):
        rs = pl.ds(i * BL, BL)
        inv = pltpu.bitcast(inv_ref[z()], BF16)
        y = jnp.dot(inv, y_s[i], preferred_element_type=F32)
        r = aq_v[t, rs, :].astype(F32) * y
        oa_v[t, rs, :] = r.astype(BF16)
        return slabs(y)

    def stage_x(t, slot):
        xu[slot] = pltpu.bitcast(x_v[t], U32)

    def mm2(lhs, li, wi, part, pi, off):
        h = D // 2
        x = pltpu.bitcast(lhs[li + z(), :, pl.ds(0, h)], BF16)
        r1 = jnp.dot(x, pltpu.bitcast(wp[wi, pl.ds(0, h // 2), :], BF16), preferred_element_type=F32)
        part[pi, pl.ds(off, TM), :] = r1
        x = pltpu.bitcast(lhs[li + z(), :, pl.ds(h, h)], BF16)
        r2 = jnp.dot(x, pltpu.bitcast(wp[wi, pl.ds(h // 2, h // 2), :], BF16), preferred_element_type=F32)
        r = part[pi + z(), pl.ds(off, TM), :] + r2
        return r, slabs(r1) + slabs(r2)

    def half_proj(sec, hf, c):
        dst, off = ((q_s, 0), (k0_s, HALO), (v_s, HALO))[sec]
        h = D // 2
        x = pltpu.bitcast(xu[z(), :, pl.ds(hf * h, h)], BF16)
        r = jnp.dot(x, pltpu.bitcast(wp[sec * 8 + c, pl.ds(hf * h // 2, h // 2), :], BF16),
                    preferred_element_type=F32)
        dst[c, pl.ds(off, TM), :] = dst[c + z(), pl.ds(off, TM), :] + r if hf else r
        return slabs(r)

    def b_proj(slot, sec, c):
        dst, off = ((q_s, 0), (k_s, HALO), (v_s, HALO))[sec]
        r, toks = mm2(xu, slot, sec * 8 + c, dst, c, off)
        dst[c, pl.ds(off, TM), :] = r
        return toks

    cexp = (DH ** -0.5) * math.log2(math.e)
    neg = -1e9 / (DH ** -0.5)
    flip = lane ^ 1

    def soft_units(t, rg):
        r0 = rg * 8
        st = {'ls': []}
        kb = k0_s if isinstance(t, int) and t == 0 else k_s

        def logits(ws):
            zi = z()
            q = [q_s[zi + c, pl.ds(r0, 8), :] for c in range(8)]
            for w in ws:
                acc = q[0] * kb[zi, pl.ds(HALO + r0 - DIL * w, 8), :]
                for c in range(1, 8):
                    acc = acc + q[c] * kb[zi + c, pl.ds(HALO + r0 - DIL * w, 8), :]
                acc = acc + pltpu.roll(acc, 64, 1)
                acc = acc + jnp.take_along_axis(acc, flip, axis=1)
                if r0 - DIL * w < 0 and not (isinstance(t, int) and t > 0):
                    acc = jnp.where(row + (t * TM + r0 - DIL * w) >= 0, acc, neg)
                st['ls'].append(acc)
            if len(st['ls']) == WIN:
                ls = st['ls']
                m = functools.reduce(jnp.maximum, ls)
                ps = [jnp.exp2((l - m) * cexp) for l in ls]
                inv_den = 1.0 / tsum(ps)
                for w in range(WIN):
                    p_s[w, pl.ds(r0, 8), :] = ps[w] * inv_den
        return [('soft', 68, P(logits, range(0, 4))), ('soft', 108, P(logits, range(4, 8)))]

    def av_units(c, dyn=True):
        def av(rbs):
            for rb in rbs:
                r0 = rb * 16
                zi = z()
                cv = zi + c if dyn else c
                acc = p_s[zi, pl.ds(r0, 16), :] * v_s[cv, pl.ds(HALO + r0, 16), :]
                for w in range(1, WIN):
                    acc = acc + p_s[zi + w, pl.ds(r0, 16), :] * v_s[cv, pl.ds(HALO + r0 - DIL * w, 16), :]
                o_s[c, pl.ds(r0, 16), :] = acc.astype(BF16)
            if rbs[-1] == TM // 16 - 1:
                ou[0, :, pl.ds(c * 128, 128)] = pltpu.bitcast(o_s[c + z()], U32)
        return [('av', 64, P(av, (rb, rb + 1))) for rb in range(0, TM // 16, 2)]

    def b_out(t, c):
        r, toks = mm2(ou, 0, 24 + c, acc_s, c % 2, 0)
        ob_v[t, :, pl.ds(c * 128, 128)] = r.astype(BF16)
        return toks

    def gate(kind, tok):
        if kind == 'conv':
            ug_s[6 * 16 * NB + zero] = tok
        elif kind == 'soft':
            q_s[8 + zero, pl.ds(0, 8), :] = tok
        elif kind == 'av':
            p_s[8 + zero, pl.ds(0, 8), :] = tok
        elif kind == 'wv':
            w_v[32 + zero, pl.ds(0, 16), :] = pltpu.bitcast(tok, BF16)
        elif kind == 'wta':
            wt_a[8 + zero, pl.ds(0, 8), :] = pltpu.bitcast(tok, U32)
        elif kind == 'wtb':
            wt_b[8 + zero, pl.ds(0, 8), :] = pltpu.bitcast(tok, U32)
        elif kind == 'prep':
            kf_s[pl.ds(pl.multiple_of(S + 8 + zero * 8, 8), 8), :] = tok

    def a_consts(t):
        cs = pl.ds(al(t, CH), CH)
        skt_all = sk_ref[:, cs].astype(F32)
        sd = jnp.sum(jnp.where(row == t, sd_ref[...].astype(F32), 0.0), axis=0, keepdims=True)
        return [skt_all[d:d + 1, :] for d in range(KS)], sd

    def halo(ref, src=None):
        ref[:, pl.ds(0, HALO), :] = (ref if src is None else src)[:, pl.ds(TM, HALO), :]

    def pace(toks, units, lead=0):
        total = sum(u[1] for u in units)
        done = 0
        last = {}
        for kind, cost, fn in units:
            i = (len(toks) + lead) * done // total - lead
            if i >= 0 and last.get(kind) != i:
                gate(kind, toks[i])
                last[kind] = i
            fn()
            done += cost

    def merge(*lists):
        items = []
        for l in lists:
            if not l:
                continue
            tot = sum(u[1] for u in l)
            acc = 0
            for u in l:
                items.append((acc / tot, len(items), u))
                acc += u[1]
        return [u for _, _, u in sorted(items, key=lambda x: x[:2])]

    def emit(units):
        for u in units:
            u[2]()

    def tiny(i):
        return pltpu.make_async_copy(w_hbm.at[pl.ds(0, 16), pl.ds(0, 128)], tiny_v.at[i], sem_w.at[32 + i])

    nstart = [0]

    def start(ws, ins):
        for t, n in ins:
            in_copy(t, n).start()
        for sec in ws:
            for n in range(8):
                wo_copy(n).start()
        tiny(nstart[0]).wait()
        nstart[0] += 1

    def w_wait(sec):
        for n in range(8):
            wo_copy(n).wait()

    def in_wait(*tn):
        for t, n in tn:
            in_copy(t, n).wait()

    def soft_rows(t, a, b):
        return [u for rg in range(a, b) for u in soft_units(t, rg)]

    def prep_pair(t, c, skt):
        return prep_units(t, 2 * c, skt) + prep_units(t, 2 * c + 1, skt)

    def dft_pair(t, c, sd):
        toks = a_inv(t, 2 * c)
        a_inv(t, 2 * c + 1)
        toks += a_fwd(t + 1, 2 * c, sd)
        a_fwd(t + 1, 2 * c + 1, sd)
        return toks

    def tail_phases(t, extra, hook=None):
        halo(k_s, k0_s if extra else None)
        conv = [u for g in range(16) for u in conv_units(g)]
        ctot = sum(u[1] for u in conv)
        cdone = 0
        cw = CONV_W1 if extra else CONV_W
        for k in range(24):
            ph, c = divmod(k, 8)
            if hook is not None and k == 8:
                hook()
            toks = b_out(t, c) if ph == 2 else b_proj((t + 1) % 2, 1 - ph, c)
            mine = []
            while conv and cdone < ctot * sum(cw[:k + 1]) / sum(cw):
                cdone += conv[0][1]
                mine.append(conv.pop(0))
            units = merge(mine, av_units(c) if ph == 0 else [], extra.get(k, []))
            if units:
                pace(toks[:TAIL] if k == 23 else toks, units)
        copy_a(t).start()
        copy_b(t).start()

    for n in range(3):
        first_copy(0, n).start()
    for i in range(NTINY):
        tiny(i).start()
    k0_s[:, pl.ds(0, HALO), :] = jnp.zeros((8, HALO, 128), F32)
    v_s[:, pl.ds(0, HALO), :] = jnp.zeros((8, HALO, 128), F32)
    kf_s[pl.ds(0, 8), :] = jnp.zeros((8, 128), F32)
    start([], [])
    for n in range(3):
        first_copy(1, n).start()
    for n in range(3):
        first_copy(0, n).wait()
    for n in range(8):
        wh_copy(0, n).start()
    start([], [(0, 3)])
    skt, sd = a_consts(0)
    for c in range(8):
        if c == 4:
            for n in range(8):
                wh_copy(1, n).start()
            for n in range(3):
                first_copy(1, n).wait()
        if c % 4 == 0:
            emit(prep_pair(0, c, skt))
        toks = a_fwd(0, 2 * c, sd)
        a_fwd(0, 2 * c + 1, sd)
        if c % 4 < 3:
            pace(toks[:12], prep_pair(0, c + 1, skt), 4)
    conv = [u for g in range(16) for u in conv_units(g)]
    per = len(conv) // 16
    emit(conv[:PRO_G[0] * per])
    nxt_in = ((1, 3), (0, 4), (1, 0), (1, 1), (1, 2))

    def ready(p):
        if p + 2 < 6:
            for n in range(8):
                wh_copy(p + 2, n).start()
        elif p == 4:
            for tn in nxt_in:
                in_copy(*tn).start()
        for n in range(8):
            wh_copy(p, n).wait()
        if p == 0:
            in_wait((0, 3))
            stage_x(0, 0)
        sec, hf = (1, 0, 2)[p // 2], p % 2
        lanes = [lane_units(sec, c)[4 * hf:4 * hf + 4] for c in range(8)]
        return sel_units(sec)[32 * hf:32 * hf + 32], lanes

    soft = soft_rows(0, 0, 32)
    fills = [conv[PRO_G[p] * per:PRO_G[p + 1] * per] for p in range(4)]
    fills += [soft[:PRO_SOFT], soft[PRO_SOFT:]]
    sel, lanes = ready(0)
    emit(sel + lanes[0] + lanes[1])
    for p in range(6):
        fill = fills[p]
        slots = (0, 1, 2, 3, 6, 7) if p < 5 else (0, 1, 2, 3, 4, 5, 6)
        for c in range(8):
            if c == 4 and p < 5:
                sel, nxt = ready(p + 1)
            toks = half_proj((1, 0, 2)[p // 2], p % 2, c)
            units = [lanes[c + 2] if c < 6 else nxt[c - 6] if p < 5 else []]
            if c in slots:
                i = slots.index(c)
                units.append(fill[len(fill) * i // len(slots):len(fill) * (i + 1) // len(slots)])
            elif p < 5:
                units.append(sel[16 * (c - 4):16 * (c - 3)])
            units = merge(*units)
            if units:
                pace(toks[:12] if c == 3 else toks, units)
        lanes = nxt
    for n in range(8):
        wo_copy(n).start()
    in_wait(*nxt_in)
    stage_x(1, 1)
    skt, sd = a_consts(1)
    emit(prep_pair(1, 0, skt))
    for e in range(8):
        toks = dft_pair(0, e, sd)
        if e < 7:
            pace(toks[:20], prep_pair(1, e + 1, skt), 4)

    def hook():
        w_wait(3)
        start([], [(1, 4), (2, 0), (2, 1), (2, 2), (2, 3)])
    tail_phases(0, {8 + c: wo_units(c) for c in range(8)}, hook)

    assert nstart[0] == NTINY

    def loop(t, carry):
        in_copy(t + 1, 4).start()

        @pl.when(t + 2 < NSTEP)
        def _():
            for n in range(4):
                in_copy(t + 2, n).start()

        in_wait((t, 4), (t + 1, 0), (t + 1, 1), (t + 1, 2), (t + 1, 3))

        halo(v_s)
        skt, sd = a_consts(t + 1)
        stage_x(t + 1, (t + 1) % 2)
        emit(prep_pair(t + 1, 0, skt))
        for c in range(8):
            toks = b_proj(t % 2, 2, c) + dft_pair(t, c, sd)
            soft = soft_rows(1, 4 * c, 4 * c + 4)
            if c < 7:
                pace(toks, merge(soft, prep_pair(t + 1, c + 1, skt)), LEAD if c == 0 else 0)
            else:
                pace(toks[:FIN], soft)
        tail_phases(t, {})
        return carry
    jax.lax.fori_loop(1, NSTEP - 1, loop, 0)

    t = NSTEP - 1
    in_wait((t, 4))
    halo(v_s)
    for c in range(8):
        toks = b_proj(t % 2, 2, c)
        if c < 5:
            pace(toks, [u for rg in range(32) if rg * 5 // 32 == c for u in soft_units(t, rg)],
                 LEAD if c == 0 else 0)
        else:
            pace(toks, [u for cc in ((0, 1), (2, 3), (4, 5))[c - 5] for u in av_units(cc, False)])
    toks = []
    for i in range(NB):
        tk = a_inv(t, i)
        if i % 2 == 0:
            toks += tk
    pace(toks[:40], av_units(6, False) + av_units(7, False))
    copy_a(t).start()
    for c in range(8):
        b_out(t, c)
        if c % 2 == 1:
            copy_b_last(c // 2).start()
    for s in range(NSTEP - 1):
        copy_a(s).wait()
        copy_b(s).wait()
    copy_a(t).wait()
    for n in range(4):
        copy_b_last(n).wait()


@jax.jit
def pallas_concat_heads__ssm_conv_h3__sliding_local_dilated__prompt_kernel(
    A_q, A_k, A_v, A_shift_k, A_ssm_k, A_ssm_D, B_x, B_wqkv, B_wo,
):
    fwd, inv = _dft_consts()
    fwd = jnp.asarray(_pack_rows(fwd))
    inv = jnp.asarray(_pack_rows(inv))
    hbm = pl.BlockSpec(memory_space=pl.ANY)
    vmem = pl.BlockSpec(memory_space=pltpu.VMEM)
    smem = pl.BlockSpec(memory_space=pltpu.SMEM)
    out = pl.pallas_call(
        _kernel,
        in_specs=[smem, hbm, hbm, hbm, vmem, hbm, vmem, hbm, hbm, hbm, vmem, vmem],
        out_specs=hbm,
        out_shape=jax.ShapeDtypeStruct((S, 2 * D), BF16),
        scratch_shapes=[
            pltpu.VMEM((NSTEP, S, CH), BF16),
            pltpu.VMEM((NSTEP, S, CH), BF16),
            pltpu.VMEM((NSTEP, S, CH), BF16),
            pltpu.VMEM((NSTEP, CH, S), BF16),
            pltpu.VMEM((NSTEP, TM, D), BF16),
            pltpu.VMEM((33, D, 128), BF16),
            pltpu.VMEM((32, D // 2, 128), U32),
            pltpu.VMEM((9, D // 2, 128), U32),
            pltpu.VMEM((9, D // 2, 128), U32),
            pltpu.VMEM((2, TM // 2, D), U32),
            pltpu.VMEM((1, TM // 2, D), U32),
            pltpu.VMEM((2, TM, 128), F32),
            pltpu.VMEM((9, TM, 128), F32),
            pltpu.VMEM((8, TM + HALO, 128), F32),
            pltpu.VMEM((8, TM + HALO, 128), F32),
            pltpu.VMEM((WIN + 1, TM, 128), F32),
            pltpu.VMEM((8, TM, 128), BF16),
            pltpu.VMEM((S + 16, 128), F32),
            pltpu.VMEM((S, 128), BF16),
            pltpu.VMEM((6 * 16 * NB + 1, 8, 128), F32),
            pltpu.VMEM((NB, 2 * BL, 128), BF16),
            pltpu.VMEM((NSTEP, S, CH), BF16),
            pltpu.VMEM((NSTEP, TM, D), BF16),
            pltpu.VMEM((NTINY, 16, 128), BF16),
            pltpu.VMEM((8, TM + HALO, 128), F32),
            pltpu.SemaphoreType.DMA((NSTEP, 5)),
            pltpu.SemaphoreType.DMA((32 + NTINY,)),
            pltpu.SemaphoreType.DMA((NSTEP, 5)),
            pltpu.SemaphoreType.DMA((NH, 3)),
            pltpu.SemaphoreType.DMA((6, 8)),
        ],
        compiler_params=pltpu.CompilerParams(vmem_limit_bytes=100 * 1024 * 1024),
    )(jnp.zeros((NZ,), jnp.int32), A_q.reshape(S, D), A_k.reshape(S, D), A_v.reshape(S, D),
      A_shift_k.T, A_ssm_k, A_ssm_D.reshape(NSTEP, CH),
      B_x.reshape(S, D), B_wqkv, B_wo, fwd, inv)
    return out.reshape(1, S, 2 * D)
```

```python
import functools
import math

import jax
import jax.numpy as jnp
import numpy as np
import jax.experimental.pallas as pl
import jax.experimental.pallas.tpu as pltpu

S = 2048
D = 1024
DH = 32
WIN = 8
DIL = 2
KS = 4
BL = 128
NB = S // BL
NSTEP = 8
TM = S // NSTEP
CH = D // NSTEP
HALO = 16
F32 = jnp.float32
BF16 = jnp.bfloat16
U32 = jnp.uint32


def _dft_consts():
    n = 2 * BL
    fwd = np.zeros((n, BL), np.float64)
    inv = np.zeros((BL, n), np.float64)
    t = np.arange(BL)
    for g in range(16):
        for r in range(8):
            f = 2 * (8 * g + r)
            ang = 2.0 * np.pi * (f + 0.5) * t / n
            fwd[16 * g + r] = np.cos(ang)
            fwd[16 * g + 8 + r] = -np.sin(ang)
            inv[:, 16 * g + r] = np.cos(ang) * (2.0 / n)
            inv[:, 16 * g + 8 + r] = -np.sin(ang) * (2.0 / n)
    return fwd.astype(np.float32), inv.astype(np.float32)


NZ = 64
NTINY = 3
NH = 2
LEAD = 8
FIN = 44
TAIL = 12
CONV_W = [3] * 8 + [8] * 15 + [3]
CONV_W1 = [4] * 8 + [6] * 8 + [9] * 7 + [3]
PRO_G = (7, 9, 11, 13, 16)
PRO_SOFT = 30


def _pack_rows(a):
    b = np.asarray(a, dtype=jnp.bfloat16).view(np.uint16).astype(np.uint32)
    return (b[0::2] | (b[1::2] << 16))[None]


def _kernel(zero_ref, aq_hbm, ak_hbm, av_hbm, sk_ref, hk_hbm, sd_ref, x_hbm, w_hbm, wo_hbm,
            fwd_ref, inv_ref, out_hbm,
            aq_v, ak_v, av_v, hk_v, x_v, w_v, wp, wt_a, wt_b,
            xu, ou, acc_s, q_s, k_s, v_s, p_s, o_s, kf_s, kv_s, ug_s, y_s, oa_v, ob_v, tiny_v, k0_s,
            sem_in, sem_w, sem_out, sem_h, sem_k):
    lane = jax.lax.broadcasted_iota(jnp.int32, (8, 128), 1)
    row = jax.lax.broadcasted_iota(jnp.int32, (8, 128), 0)
    zero = zero_ref[0]
    zcount = [0]
    P = functools.partial

    def z():
        zcount[0] = zcount[0] % (NZ - 1) + 1
        return zero_ref[zcount[0]]

    def al(i, m):
        return i * m if isinstance(i, int) else pl.multiple_of(i * m, m)

    def in_copy(t, n):
        cs = pl.ds(al(t, CH), CH)
        rs = pl.ds(al(t, TM), TM)
        if n == 0:
            src, dst = ak_hbm.at[:, cs], ak_v
        elif n == 1:
            src, dst = av_hbm.at[:, cs], av_v
        elif n == 2:
            src, dst = hk_hbm.at[cs, :], hk_v
        elif n == 3:
            src, dst = x_hbm.at[rs, :], x_v
        else:
            src, dst = aq_hbm.at[:, cs], aq_v
        return pltpu.make_async_copy(src, dst.at[t], sem_in.at[t, n])

    def first_copy(h, n):
        ts = pl.ds(h * (S // NH), S // NH)
        cs = pl.ds(0, CH)
        if n == 2:
            src, dst = hk_hbm.at[cs, ts], hk_v.at[0, :, ts]
        else:
            src, dst = (ak_hbm, av_hbm)[n].at[ts, cs], (ak_v, av_v)[n].at[0, ts, :]
        return pltpu.make_async_copy(src, dst, sem_h.at[h, n])

    def wh_copy(p, n):
        col = (8, 0, 16)[p // 2] + n
        rs = pl.ds((p % 2) * (D // 2), D // 2)
        return pltpu.make_async_copy(w_hbm.at[rs, pl.ds(col * 128, 128)], w_v.at[col, rs, :],
                                     sem_k.at[p, n])

    def wo_copy(n):
        return pltpu.make_async_copy(wo_hbm.at[:, pl.ds(n * 128, 128)], w_v.at[24 + n], sem_w.at[24 + n])

    def copy_a(t):
        return pltpu.make_async_copy(oa_v.at[t], out_hbm.at[:, pl.ds(al(t, CH), CH)], sem_out.at[t, 0])

    def copy_b(t):
        return pltpu.make_async_copy(
            ob_v.at[t], out_hbm.at[pl.ds(al(t, TM), TM), pl.ds(D, D)], sem_out.at[t, 1])

    def copy_b_last(n):
        t = NSTEP - 1
        return pltpu.make_async_copy(
            ob_v.at[t, :, pl.ds(n * 256, 256)],
            out_hbm.at[pl.ds(t * TM, TM), pl.ds(D + n * 256, 256)], sem_out.at[t, 1 + n])

    def xor_select(c, sel):
        for s in range(3):
            bit = (sel & (1 << s)) != 0
            c = [jnp.where(bit, c[i ^ (1 << s)], c[i]) for i in range(8)]
        return c

    def tsum(vals):
        return functools.reduce(lambda a, b: a + b, vals)

    def lane_src(j):
        return (((lane >> 4) & 3) << 5) | ((lane >> 6) << 4) | ((((lane >> 1) & 7) ^ j) << 1) | (lane & 1)

    def wtmp(sec):
        return (wt_b, wt_a, wt_a)[sec], ('wtb', 'wta', 'wta')[sec]

    def sel_units(sec):
        wt, _ = wtmp(sec)

        def sel(rb):
            c = [pltpu.bitcast(w_v[sec * 8 + i, pl.ds(rb * 16, 16), :], U32) for i in range(8)]
            c = xor_select(c, lane >> 1)
            for j in range(8):
                wt[j, pl.ds(rb * 8, 8), :] = c[j]
        return [('wv', 32, P(sel, rb)) for rb in range(64)]

    def lane_units(sec, j):
        wt, kind = wtmp(sec)

        def lanes(rb):
            zi = z()
            for r in range(rb * 64, rb * 64 + 64, 8):
                wp[sec * 8 + j, pl.ds(r, 8), :] = jnp.take_along_axis(
                    wt[zi + j, pl.ds(r, 8), :], lane_src(j), axis=1)
        return [(kind, 32, P(lanes, rb)) for rb in range(8)]

    def wo_units(c):
        def rows(mp):
            m = ((mp & 3) << 1) | (mp >> 2)
            tr = [pltpu.bitcast(w_v[24 + c, pl.ds(r * 128 + m * 16, 16), :], U32) for r in range(8)]
            tr = xor_select(tr, row)
            for j in range(8):
                wp[24 + c, pl.ds(j * 64 + mp * 8, 8), :] = (
                    jnp.take_along_axis(tr[j], row ^ j, axis=0) if j else tr[j])
        return [('wv', 40, P(rows, mp)) for mp in range(8)]

    def a_prep(t, r0, n, skt):
        kf_s[pl.ds(8 + r0, n), :] = ak_v[t, pl.ds(r0, n), :].astype(F32)
        ksh = kf_s[pl.ds(8 + r0, n), :] * skt[0]
        for d in range(1, KS):
            ksh = ksh + kf_s[pl.ds(8 + r0 - d, n), :] * skt[d]
        kv_s[pl.ds(r0, n), :] = (ksh * av_v[t, pl.ds(r0, n), :].astype(F32)).astype(BF16)

    def prep_units(t, j, skt):
        return [('prep', 48, P(a_prep, t, j * BL + r, 32, skt)) for r in range(0, BL, 32)]

    def slabs(r):
        return [r[i:i + 8] for i in range(0, r.shape[0], 16)]

    def ug(plane, g, j):
        return (plane * 16 + g) * NB + j

    def a_fwd(t, j, sd):
        fwd = pltpu.bitcast(fwd_ref[z()], BF16)
        u = jnp.dot(fwd, kv_s[pl.ds(j * BL, BL), :], preferred_element_type=F32)
        fwd = pltpu.bitcast(fwd_ref[z()], BF16)
        h = jax.lax.dot_general(fwd, hk_v[t, :, pl.ds(j * BL, BL)],
                                (((1,), (1,)), ((), ())), preferred_element_type=F32)
        for g in range(16):
            ur, ui = u[16 * g:16 * g + 8], u[16 * g + 8:16 * g + 16]
            ug_s[ug(0, g, j)] = ur + ui
            ug_s[ug(1, g, j)] = ur
            ug_s[ug(2, g, j)] = ui
            hr, hi = h[16 * g:16 * g + 8], h[16 * g + 8:16 * g + 16]
            if j == 0:
                hr = hr + sd
            ug_s[ug(3, g, j)] = hr
            ug_s[ug(4, g, j)] = hi - hr
            ug_s[ug(5, g, j)] = hr + hi
        return slabs(u)

    def conv_units(g):
        st = {'prev': None}

        def toep(ib, pl_):
            zi = z()
            acc = [None] * 4 if pl_ == 0 else list(st[0])
            gs = {}
            for jb in range(ib + 1):
                us = [ug_s[zi + ug(pl_, g, 4 * jb + b)] for b in range(4)]
                m0 = 4 * (ib - jb)
                gs = {m: gs[m] if m in gs else ug_s[zi + ug(3 + pl_, g, m)]
                      for m in range(max(m0 - 3, 0), m0 + 4)}
                for a in range(4):
                    for b in range(4):
                        m = m0 + a - b
                        if m < 0:
                            continue
                        pr = us[b] * gs[m]
                        if acc[a] is None:
                            acc[a] = pr
                        else:
                            acc[a] = acc[a] + pr if pl_ < 2 else acc[a] - pr
            st[pl_] = acc
            if pl_ == 2:
                im, re = st[1], st[2]
                for a in range(4):
                    prev = st['prev']
                    if prev is None:
                        yr, yi = re[a], im[a]
                    else:
                        yr, yi = re[a] - prev[1], im[a] + prev[0]
                    st['prev'] = (re[a], im[a])
                    y_s[4 * ib + a, pl.ds(16 * g, 16), :] = jnp.concatenate([yr, yi], axis=0).astype(BF16)
        return [('conv', 20 + 32 * ib + (12 if pl_ == 2 else 0), P(toep, ib, pl_))
                for ib in range(4) for pl_ in range(3)]

    def a_conv(g):
        for _, _, fn in conv_units(g):
            fn()

    def a_inv(t, i):
        rs = pl.ds(i * BL, BL)
        inv = pltpu.bitcast(inv_ref[z()], BF16)
        y = jnp.dot(inv, y_s[i], preferred_element_type=F32)
        r = aq_v[t, rs, :].astype(F32) * y
        oa_v[t, rs, :] = r.astype(BF16)
        return slabs(y)

    def stage_x(t, slot):
        xu[slot] = pltpu.bitcast(x_v[t], U32)

    def mm2(lhs, li, wi, part, pi, off):
        h = D // 2
        x = pltpu.bitcast(lhs[li + z(), :, pl.ds(0, h)], BF16)
        r1 = jnp.dot(x, pltpu.bitcast(wp[wi, pl.ds(0, h // 2), :], BF16), preferred_element_type=F32)
        part[pi, pl.ds(off, TM), :] = r1
        x = pltpu.bitcast(lhs[li + z(), :, pl.ds(h, h)], BF16)
        r2 = jnp.dot(x, pltpu.bitcast(wp[wi, pl.ds(h // 2, h // 2), :], BF16), preferred_element_type=F32)
        r = part[pi + z(), pl.ds(off, TM), :] + r2
        return r, slabs(r1) + slabs(r2)

    def half_proj(sec, hf, c):
        dst, off = ((q_s, 0), (k0_s, HALO), (v_s, HALO))[sec]
        h = D // 2
        x = pltpu.bitcast(xu[z(), :, pl.ds(hf * h, h)], BF16)
        r = jnp.dot(x, pltpu.bitcast(wp[sec * 8 + c, pl.ds(hf * h // 2, h // 2), :], BF16),
                    preferred_element_type=F32)
        dst[c, pl.ds(off, TM), :] = dst[c + z(), pl.ds(off, TM), :] + r if hf else r
        return slabs(r)

    def b_proj(slot, sec, c):
        dst, off = ((q_s, 0), (k_s, HALO), (v_s, HALO))[sec]
        r, toks = mm2(xu, slot, sec * 8 + c, dst, c, off)
        dst[c, pl.ds(off, TM), :] = r
        return toks

    cexp = (DH ** -0.5) * math.log2(math.e)
    neg = -1e9 / (DH ** -0.5)
    flip = lane ^ 1

    def soft_units(t, rg):
        r0 = rg * 8
        st = {'ls': []}
        kb = k0_s if isinstance(t, int) and t == 0 else k_s

        def logits(ws):
            zi = z()
            q = [q_s[zi + c, pl.ds(r0, 8), :] for c in range(8)]
            for w in ws:
                acc = q[0] * kb[zi, pl.ds(HALO + r0 - DIL * w, 8), :]
                for c in range(1, 8):
                    acc = acc + q[c] * kb[zi + c, pl.ds(HALO + r0 - DIL * w, 8), :]
                acc = acc + pltpu.roll(acc, 64, 1)
                acc = acc + jnp.take_along_axis(acc, flip, axis=1)
                if r0 - DIL * w < 0 and not (isinstance(t, int) and t > 0):
                    acc = jnp.where(row + (t * TM + r0 - DIL * w) >= 0, acc, neg)
                st['ls'].append(acc)
            if len(st['ls']) == WIN:
                ls = st['ls']
                m = functools.reduce(jnp.maximum, ls)
                ps = [jnp.exp2((l - m) * cexp) for l in ls]
                inv_den = 1.0 / tsum(ps)
                for w in range(WIN):
                    p_s[w, pl.ds(r0, 8), :] = ps[w] * inv_den
        return [('soft', 68, P(logits, range(0, 4))), ('soft', 108, P(logits, range(4, 8)))]

    def av_units(c, dyn=True):
        def av(rbs):
            for rb in rbs:
                r0 = rb * 16
                zi = z()
                cv = zi + c if dyn else c
                acc = p_s[zi, pl.ds(r0, 16), :] * v_s[cv, pl.ds(HALO + r0, 16), :]
                for w in range(1, WIN):
                    acc = acc + p_s[zi + w, pl.ds(r0, 16), :] * v_s[cv, pl.ds(HALO + r0 - DIL * w, 16), :]
                o_s[c, pl.ds(r0, 16), :] = acc.astype(BF16)
            if rbs[-1] == TM // 16 - 1:
                ou[0, :, pl.ds(c * 128, 128)] = pltpu.bitcast(o_s[c + z()], U32)
        return [('av', 64, P(av, (rb, rb + 1))) for rb in range(0, TM // 16, 2)]

    def b_out(t, c):
        r, toks = mm2(ou, 0, 24 + c, acc_s, c % 2, 0)
        ob_v[t, :, pl.ds(c * 128, 128)] = r.astype(BF16)
        return toks

    def gate(kind, tok):
        if kind == 'conv':
            ug_s[6 * 16 * NB + zero] = tok
        elif kind == 'x':
            x_v[NSTEP + zero, pl.ds(0, 16), pl.ds(0, 128)] = pltpu.bitcast(tok, BF16)
        elif kind == 'soft':
            q_s[8 + zero, pl.ds(0, 8), :] = tok
        elif kind == 'av':
            p_s[8 + zero, pl.ds(0, 8), :] = tok
        elif kind == 'wv':
            w_v[32 + zero, pl.ds(0, 16), :] = pltpu.bitcast(tok, BF16)
        elif kind == 'wta':
            wt_a[8 + zero, pl.ds(0, 8), :] = pltpu.bitcast(tok, U32)
        elif kind == 'wtb':
            wt_b[8 + zero, pl.ds(0, 8), :] = pltpu.bitcast(tok, U32)
        elif kind == 'prep':
            kf_s[pl.ds(pl.multiple_of(S + 8 + zero * 8, 8), 8), :] = tok

    def a_consts(t):
        cs = pl.ds(al(t, CH), CH)
        skt_all = sk_ref[:, cs].astype(F32)
        sd = jnp.sum(jnp.where(row == t, sd_ref[...].astype(F32), 0.0), axis=0, keepdims=True)
        return [skt_all[d:d + 1, :] for d in range(KS)], sd

    def halo(ref, src=None):
        ref[:, pl.ds(0, HALO), :] = (ref if src is None else src)[:, pl.ds(TM, HALO), :]

    def pace(toks, units, lead=0):
        total = sum(u[1] for u in units)
        done = 0
        last = {}
        for kind, cost, fn in units:
            i = (len(toks) + lead) * done // total - lead
            if i >= 0 and last.get(kind) != i:
                gate(kind, toks[i])
                last[kind] = i
            fn()
            done += cost

    def merge(*lists):
        items = []
        for l in lists:
            if not l:
                continue
            tot = sum(u[1] for u in l)
            acc = 0
            for u in l:
                items.append((acc / tot, len(items), u))
                acc += u[1]
        return [u for _, _, u in sorted(items, key=lambda x: x[:2])]

    def emit(units):
        for u in units:
            u[2]()

    def tiny(i):
        return pltpu.make_async_copy(w_hbm.at[pl.ds(0, 16), pl.ds(0, 128)], tiny_v.at[i], sem_w.at[32 + i])

    nstart = [0]

    def start(ws, ins):
        for t, n in ins:
            in_copy(t, n).start()
        for sec in ws:
            for n in range(8):
                wo_copy(n).start()
        tiny(nstart[0]).wait()
        nstart[0] += 1

    def w_wait(sec):
        for n in range(8):
            wo_copy(n).wait()

    def in_wait(*tn):
        for t, n in tn:
            in_copy(t, n).wait()

    def soft_rows(t, a, b):
        return [u for rg in range(a, b) for u in soft_units(t, rg)]

    def prep_pair(t, c, skt):
        return prep_units(t, 2 * c, skt) + prep_units(t, 2 * c + 1, skt)

    def dft_pair(t, c, sd):
        toks = a_inv(t, 2 * c)
        a_inv(t, 2 * c + 1)
        toks += a_fwd(t + 1, 2 * c, sd)
        a_fwd(t + 1, 2 * c + 1, sd)
        return toks

    def tail_phases(t, extra, hook=None):
        halo(k_s, k0_s if extra else None)
        conv = [u for g in range(16) for u in conv_units(g)]
        ctot = sum(u[1] for u in conv)
        cdone = 0
        cw = CONV_W1 if extra else CONV_W
        for k in range(24):
            ph, c = divmod(k, 8)
            if hook is not None and k == 8:
                hook()
            toks = b_out(t, c) if ph == 2 else b_proj((t + 1) % 2, 1 - ph, c)
            if ph == 2:
                gate('x', toks[4])
                t2 = t + 2 if isinstance(t, int) else jnp.minimum(t + 2, NSTEP - 1)
                xu[t % 2, pl.ds(16 * c, 16), :] = pltpu.bitcast(x_v[t2, pl.ds(32 * c, 32), :], U32)
            mine = []
            while conv and cdone < ctot * sum(cw[:k + 1]) / sum(cw):
                cdone += conv[0][1]
                mine.append(conv.pop(0))
            units = merge(mine, av_units(c) if ph == 0 else [], extra.get(k, []))
            if units:
                pace(toks[:TAIL] if k == 23 else toks, units)
        copy_a(t).start()
        copy_b(t).start()

    for n in range(3):
        first_copy(0, n).start()
    for i in range(NTINY):
        tiny(i).start()
    k0_s[:, pl.ds(0, HALO), :] = jnp.zeros((8, HALO, 128), F32)
    v_s[:, pl.ds(0, HALO), :] = jnp.zeros((8, HALO, 128), F32)
    kf_s[pl.ds(0, 8), :] = jnp.zeros((8, 128), F32)
    start([], [])
    for n in range(3):
        first_copy(1, n).start()
    for n in range(3):
        first_copy(0, n).wait()
    for n in range(8):
        wh_copy(0, n).start()
    start([], [(0, 3)])
    skt, sd = a_consts(0)
    for c in range(8):
        if c == 4:
            for n in range(8):
                wh_copy(1, n).start()
            for n in range(3):
                first_copy(1, n).wait()
        if c % 4 == 0:
            emit(prep_pair(0, c, skt))
        toks = a_fwd(0, 2 * c, sd)
        a_fwd(0, 2 * c + 1, sd)
        if c % 4 < 3:
            pace(toks[:12], prep_pair(0, c + 1, skt), 4)
    conv = [u for g in range(16) for u in conv_units(g)]
    per = len(conv) // 16
    emit(conv[:PRO_G[0] * per])
    nxt_in = ((1, 3), (0, 4), (1, 0), (1, 1), (1, 2))

    def ready(p):
        if p + 2 < 6:
            for n in range(8):
                wh_copy(p + 2, n).start()
        elif p == 4:
            for tn in nxt_in:
                in_copy(*tn).start()
        for n in range(8):
            wh_copy(p, n).wait()
        if p == 0:
            in_wait((0, 3))
            stage_x(0, 0)
        sec, hf = (1, 0, 2)[p // 2], p % 2
        lanes = [lane_units(sec, c)[4 * hf:4 * hf + 4] for c in range(8)]
        return sel_units(sec)[32 * hf:32 * hf + 32], lanes

    soft = soft_rows(0, 0, 32)
    fills = [conv[PRO_G[p] * per:PRO_G[p + 1] * per] for p in range(4)]
    fills += [soft[:PRO_SOFT], soft[PRO_SOFT:]]
    sel, lanes = ready(0)
    emit(sel + lanes[0] + lanes[1])
    for p in range(6):
        fill = fills[p]
        slots = (0, 1, 2, 3, 6, 7) if p < 5 else (0, 1, 2, 3, 4, 5, 6)
        for c in range(8):
            if c == 4 and p < 5:
                sel, nxt = ready(p + 1)
            toks = half_proj((1, 0, 2)[p // 2], p % 2, c)
            units = [lanes[c + 2] if c < 6 else nxt[c - 6] if p < 5 else []]
            if c in slots:
                i = slots.index(c)
                units.append(fill[len(fill) * i // len(slots):len(fill) * (i + 1) // len(slots)])
            elif p < 5:
                units.append(sel[16 * (c - 4):16 * (c - 3)])
            units = merge(*units)
            if units:
                pace(toks[:12] if c == 3 else toks, units)
        lanes = nxt
    for n in range(8):
        wo_copy(n).start()
    in_copy(2, 3).start()
    in_wait(*nxt_in)
    stage_x(1, 1)
    skt, sd = a_consts(1)
    emit(prep_pair(1, 0, skt))
    for e in range(8):
        toks = dft_pair(0, e, sd)
        if e < 7:
            pace(toks[:20], prep_pair(1, e + 1, skt), 4)

    def hook():
        w_wait(3)
        in_wait((2, 3))
        start([], [(1, 4), (2, 0), (2, 1), (2, 2), (3, 3)])
    tail_phases(0, {8 + c: wo_units(c) for c in range(8)}, hook)

    assert nstart[0] == NTINY

    def loop(t, carry):
        in_copy(t + 1, 4).start()

        @pl.when(t + 3 < NSTEP)
        def _():
            in_copy(t + 3, 3).start()

        @pl.when(t + 2 < NSTEP)
        def _():
            for n in range(3):
                in_copy(t + 2, n).start()
            in_wait((t + 2, 3))

        in_wait((t, 4), (t + 1, 0), (t + 1, 1), (t + 1, 2))

        halo(v_s)
        skt, sd = a_consts(t + 1)
        for c in range(8):
            toks = b_proj(t % 2, 2, c)
            if c == 0:
                pace(toks[:16], prep_pair(t + 1, 0, skt), 2)
            toks = toks + dft_pair(t, c, sd)
            soft = soft_rows(1, 4 * c, 4 * c + 4)
            if c < 7:
                pace(toks, merge(soft, prep_pair(t + 1, c + 1, skt)), LEAD if c == 0 else 0)
            else:
                pace(toks[:FIN], soft)
        tail_phases(t, {})
        return carry
    jax.lax.fori_loop(1, NSTEP - 1, loop, 0)

    t = NSTEP - 1
    in_wait((t, 4))
    halo(v_s)
    for c in range(8):
        toks = b_proj(t % 2, 2, c)
        if c < 5:
            pace(toks, [u for rg in range(32) if rg * 5 // 32 == c for u in soft_units(t, rg)],
                 LEAD if c == 0 else 0)
        else:
            pace(toks, [u for cc in ((0, 1), (2, 3), (4, 5))[c - 5] for u in av_units(cc, False)])
    toks = []
    for i in range(NB):
        tk = a_inv(t, i)
        if i % 2 == 0:
            toks += tk
    pace(toks[:40], av_units(6, False) + av_units(7, False))
    copy_a(t).start()
    for c in range(8):
        b_out(t, c)
        if c % 2 == 1:
            copy_b_last(c // 2).start()
    for s in range(NSTEP - 1):
        copy_a(s).wait()
        copy_b(s).wait()
    copy_a(t).wait()
    for n in range(4):
        copy_b_last(n).wait()


@jax.jit
def pallas_concat_heads__ssm_conv_h3__sliding_local_dilated__prompt_kernel(
    A_q, A_k, A_v, A_shift_k, A_ssm_k, A_ssm_D, B_x, B_wqkv, B_wo,
):
    fwd, inv = _dft_consts()
    fwd = jnp.asarray(_pack_rows(fwd))
    inv = jnp.asarray(_pack_rows(inv))
    hbm = pl.BlockSpec(memory_space=pl.ANY)
    vmem = pl.BlockSpec(memory_space=pltpu.VMEM)
    smem = pl.BlockSpec(memory_space=pltpu.SMEM)
    out = pl.pallas_call(
        _kernel,
        in_specs=[smem, hbm, hbm, hbm, vmem, hbm, vmem, hbm, hbm, hbm, vmem, vmem],
        out_specs=hbm,
        out_shape=jax.ShapeDtypeStruct((S, 2 * D), BF16),
        scratch_shapes=[
            pltpu.VMEM((NSTEP, S, CH), BF16),
            pltpu.VMEM((NSTEP, S, CH), BF16),
            pltpu.VMEM((NSTEP, S, CH), BF16),
            pltpu.VMEM((NSTEP, CH, S), BF16),
            pltpu.VMEM((NSTEP + 1, TM, D), BF16),
            pltpu.VMEM((33, D, 128), BF16),
            pltpu.VMEM((32, D // 2, 128), U32),
            pltpu.VMEM((9, D // 2, 128), U32),
            pltpu.VMEM((9, D // 2, 128), U32),
            pltpu.VMEM((2, TM // 2, D), U32),
            pltpu.VMEM((1, TM // 2, D), U32),
            pltpu.VMEM((2, TM, 128), F32),
            pltpu.VMEM((9, TM, 128), F32),
            pltpu.VMEM((8, TM + HALO, 128), F32),
            pltpu.VMEM((8, TM + HALO, 128), F32),
            pltpu.VMEM((WIN + 1, TM, 128), F32),
            pltpu.VMEM((8, TM, 128), BF16),
            pltpu.VMEM((S + 16, 128), F32),
            pltpu.VMEM((S, 128), BF16),
            pltpu.VMEM((6 * 16 * NB + 1, 8, 128), F32),
            pltpu.VMEM((NB, 2 * BL, 128), BF16),
            pltpu.VMEM((NSTEP, S, CH), BF16),
            pltpu.VMEM((NSTEP, TM, D), BF16),
            pltpu.VMEM((NTINY, 16, 128), BF16),
            pltpu.VMEM((8, TM + HALO, 128), F32),
            pltpu.SemaphoreType.DMA((NSTEP, 5)),
            pltpu.SemaphoreType.DMA((32 + NTINY,)),
            pltpu.SemaphoreType.DMA((NSTEP, 5)),
            pltpu.SemaphoreType.DMA((NH, 3)),
            pltpu.SemaphoreType.DMA((6, 8)),
        ],
        compiler_params=pltpu.CompilerParams(vmem_limit_bytes=100 * 1024 * 1024),
    )(jnp.zeros((NZ,), jnp.int32), A_q.reshape(S, D), A_k.reshape(S, D), A_v.reshape(S, D),
      A_shift_k.T, A_ssm_k, A_ssm_D.reshape(NSTEP, CH),
      B_x.reshape(S, D), B_wqkv, B_wo, fwd, inv)
    return out.reshape(1, S, 2 * D)
```

```python
import functools
import math

import jax
import jax.numpy as jnp
import numpy as np
import jax.experimental.pallas as pl
import jax.experimental.pallas.tpu as pltpu

S = 2048
D = 1024
DH = 32
WIN = 8
DIL = 2
KS = 4
BL = 128
NB = S // BL
NSTEP = 8
TM = S // NSTEP
CH = D // NSTEP
HALO = 16
F32 = jnp.float32
BF16 = jnp.bfloat16
U32 = jnp.uint32


def _dft_consts():
    n = 2 * BL
    fwd = np.zeros((n, BL), np.float64)
    inv = np.zeros((BL, n), np.float64)
    t = np.arange(BL)
    for g in range(16):
        for r in range(8):
            f = 2 * (8 * g + r)
            ang = 2.0 * np.pi * (f + 0.5) * t / n
            fwd[16 * g + r] = np.cos(ang)
            fwd[16 * g + 8 + r] = -np.sin(ang)
            inv[:, 16 * g + r] = np.cos(ang) * (2.0 / n)
            inv[:, 16 * g + 8 + r] = -np.sin(ang) * (2.0 / n)
    return fwd.astype(np.float32), inv.astype(np.float32)


NZ = 64
NTINY = 3
NH = 2
LEAD = 4
FIN = 44
TAIL = 12
CONV_W = [3] * 8 + [8] * 15 + [3]
CONV_W1 = [4] * 8 + [6] * 8 + [9] * 7 + [3]
PRO_G = (7, 9, 11, 13, 16)
PRO_SOFT = 30


def _pack_rows(a):
    b = np.asarray(a, dtype=jnp.bfloat16).view(np.uint16).astype(np.uint32)
    return (b[0::2] | (b[1::2] << 16))[None]


def _kernel(zero_hbm, aq_hbm, ak_hbm, av_hbm, sk_hbm, hk_hbm, sd_hbm, x_hbm, w_hbm, wo_hbm,
            fwd_hbm, inv_hbm, out_hbm,
            aq_v, ak_v, av_v, hk_v, x_v, w_v, wp, wt_a, wt_b,
            xu, ou, acc_s, q_s, k_s, v_s, p_s, o_s, kf_s, kv_s, ug_s, y_s, oa_v, ob_v, tiny_v, k0_s,
            sem_in, sem_w, sem_out, sem_h, sem_k,
            sk_ref, sd_ref, fwd_ref, inv_ref, sem_c, zero_ref):
    lane = jax.lax.broadcasted_iota(jnp.int32, (8, 128), 1)
    row = jax.lax.broadcasted_iota(jnp.int32, (8, 128), 0)
    zcount = [0]
    P = functools.partial

    def z():
        zcount[0] = zcount[0] % (NZ - 1) + 1
        return zero_ref[zcount[0]]

    def al(i, m):
        return i * m if isinstance(i, int) else pl.multiple_of(i * m, m)

    def in_copy(t, n):
        cs = pl.ds(al(t, CH), CH)
        rs = pl.ds(al(t, TM), TM)
        if n == 0:
            src, dst = ak_hbm.at[:, cs], ak_v
        elif n == 1:
            src, dst = av_hbm.at[:, cs], av_v
        elif n == 2:
            src, dst = hk_hbm.at[cs, :], hk_v
        elif n == 3:
            src, dst = x_hbm.at[rs, :], x_v
        else:
            src, dst = aq_hbm.at[:, cs], aq_v
        return pltpu.make_async_copy(src, dst.at[t], sem_in.at[t, n])

    def first_copy(h, n):
        ts = pl.ds(h * (S // NH), S // NH)
        cs = pl.ds(0, CH)
        if n == 2:
            src, dst = hk_hbm.at[cs, ts], hk_v.at[0, :, ts]
        else:
            src, dst = (ak_hbm, av_hbm)[n].at[ts, cs], (ak_v, av_v)[n].at[0, ts, :]
        return pltpu.make_async_copy(src, dst, sem_h.at[h, n])

    def wh_copy(p, n):
        col = (8, 0, 16)[p // 2] + n
        rs = pl.ds((p % 2) * (D // 2), D // 2)
        return pltpu.make_async_copy(w_hbm.at[rs, pl.ds(col * 128, 128)], w_v.at[col, rs, :],
                                     sem_k.at[p, n])

    def wo_copy(n):
        return pltpu.make_async_copy(wo_hbm.at[:, pl.ds(n * 128, 128)], w_v.at[24 + n], sem_w.at[24 + n])

    def copy_a(t):
        return pltpu.make_async_copy(oa_v.at[t], out_hbm.at[:, pl.ds(al(t, CH), CH)], sem_out.at[t, 0])

    def copy_b(t):
        return pltpu.make_async_copy(
            ob_v.at[t], out_hbm.at[pl.ds(al(t, TM), TM), pl.ds(D, D)], sem_out.at[t, 1])

    def copy_b_last(n):
        t = NSTEP - 1
        return pltpu.make_async_copy(
            ob_v.at[t, :, pl.ds(n * 256, 256)],
            out_hbm.at[pl.ds(t * TM, TM), pl.ds(D + n * 256, 256)], sem_out.at[t, 1 + n])

    def xor_select(c, sel):
        for s in range(3):
            bit = (sel & (1 << s)) != 0
            c = [jnp.where(bit, c[i ^ (1 << s)], c[i]) for i in range(8)]
        return c

    def tsum(vals):
        return functools.reduce(lambda a, b: a + b, vals)

    def lane_src(j):
        return (((lane >> 4) & 3) << 5) | ((lane >> 6) << 4) | ((((lane >> 1) & 7) ^ j) << 1) | (lane & 1)

    def wtmp(sec):
        return (wt_b, wt_a, wt_a)[sec], ('wtb', 'wta', 'wta')[sec]

    def sel_units(sec):
        wt, _ = wtmp(sec)

        def sel(rb):
            c = [pltpu.bitcast(w_v[sec * 8 + i, pl.ds(rb * 16, 16), :], U32) for i in range(8)]
            c = xor_select(c, lane >> 1)
            for j in range(8):
                wt[j, pl.ds(rb * 8, 8), :] = c[j]
        return [('wv', 32, P(sel, rb)) for rb in range(64)]

    def lane_units(sec, j):
        wt, kind = wtmp(sec)

        def lanes(rb):
            zi = z()
            for r in range(rb * 64, rb * 64 + 64, 8):
                wp[sec * 8 + j, pl.ds(r, 8), :] = jnp.take_along_axis(
                    wt[zi + j, pl.ds(r, 8), :], lane_src(j), axis=1)
        return [(kind, 32, P(lanes, rb)) for rb in range(8)]

    def wo_units(c):
        def rows(mp):
            m = ((mp & 3) << 1) | (mp >> 2)
            tr = [pltpu.bitcast(w_v[24 + c, pl.ds(r * 128 + m * 16, 16), :], U32) for r in range(8)]
            tr = xor_select(tr, row)
            for j in range(8):
                wp[24 + c, pl.ds(j * 64 + mp * 8, 8), :] = (
                    jnp.take_along_axis(tr[j], row ^ j, axis=0) if j else tr[j])
        return [('wv', 40, P(rows, mp)) for mp in range(8)]

    def a_prep(t, r0, n, skt):
        kf_s[pl.ds(8 + r0, n), :] = ak_v[t, pl.ds(r0, n), :].astype(F32)
        ksh = kf_s[pl.ds(8 + r0, n), :] * skt[0]
        for d in range(1, KS):
            ksh = ksh + kf_s[pl.ds(8 + r0 - d, n), :] * skt[d]
        kv_s[pl.ds(r0, n), :] = (ksh * av_v[t, pl.ds(r0, n), :].astype(F32)).astype(BF16)

    def prep_units(t, j, skt):
        return [('prep', 48, P(a_prep, t, j * BL + r, 32, skt)) for r in range(0, BL, 32)]

    def slabs(r):
        return [r[i:i + 8] for i in range(0, r.shape[0], 16)]

    def ug(plane, g, j):
        return (plane * 16 + g) * NB + j

    def a_fwd(t, j, sd):
        fwd = pltpu.bitcast(fwd_ref[z()], BF16)
        u = jnp.dot(fwd, kv_s[pl.ds(j * BL, BL), :], preferred_element_type=F32)
        fwd = pltpu.bitcast(fwd_ref[z()], BF16)
        h = jax.lax.dot_general(fwd, hk_v[t, :, pl.ds(j * BL, BL)],
                                (((1,), (1,)), ((), ())), preferred_element_type=F32)
        for g in range(16):
            ur, ui = u[16 * g:16 * g + 8], u[16 * g + 8:16 * g + 16]
            ug_s[ug(0, g, j)] = ur + ui
            ug_s[ug(1, g, j)] = ur
            ug_s[ug(2, g, j)] = ui
            hr, hi = h[16 * g:16 * g + 8], h[16 * g + 8:16 * g + 16]
            if j == 0:
                hr = hr + sd
            ug_s[ug(3, g, j)] = hr
            ug_s[ug(4, g, j)] = hi - hr
            ug_s[ug(5, g, j)] = hr + hi
        return slabs(u)

    def conv_units(g):
        st = {'prev': None}

        def toep(ib, pl_):
            zi = z()
            acc = [None] * 4 if pl_ == 0 else list(st[0])
            gs = {}
            for jb in range(ib + 1):
                us = [ug_s[zi + ug(pl_, g, 4 * jb + b)] for b in range(4)]
                m0 = 4 * (ib - jb)
                gs = {m: gs[m] if m in gs else ug_s[zi + ug(3 + pl_, g, m)]
                      for m in range(max(m0 - 3, 0), m0 + 4)}
                for a in range(4):
                    for b in range(4):
                        m = m0 + a - b
                        if m < 0:
                            continue
                        pr = us[b] * gs[m]
                        if acc[a] is None:
                            acc[a] = pr
                        else:
                            acc[a] = acc[a] + pr if pl_ < 2 else acc[a] - pr
            st[pl_] = acc
            if pl_ == 2:
                im, re = st[1], st[2]
                for a in range(4):
                    prev = st['prev']
                    if prev is None:
                        yr, yi = re[a], im[a]
                    else:
                        yr, yi = re[a] - prev[1], im[a] + prev[0]
                    st['prev'] = (re[a], im[a])
                    y_s[4 * ib + a, pl.ds(16 * g, 16), :] = jnp.concatenate([yr, yi], axis=0).astype(BF16)
        return [('conv', 20 + 32 * ib + (12 if pl_ == 2 else 0), P(toep, ib, pl_))
                for ib in range(4) for pl_ in range(3)]

    def a_conv(g):
        for _, _, fn in conv_units(g):
            fn()

    def a_inv(t, i):
        rs = pl.ds(i * BL, BL)
        inv = pltpu.bitcast(inv_ref[z()], BF16)
        y = jnp.dot(inv, y_s[i], preferred_element_type=F32)
        r = aq_v[t, rs, :].astype(F32) * y
        oa_v[t, rs, :] = r.astype(BF16)
        return slabs(y)

    def stage_x(t, slot):
        xu[slot] = pltpu.bitcast(x_v[t], U32)

    def mm2(lhs, li, wi, part, pi, off):
        h = D // 2
        x = pltpu.bitcast(lhs[li + z(), :, pl.ds(0, h)], BF16)
        r1 = jnp.dot(x, pltpu.bitcast(wp[wi, pl.ds(0, h // 2), :], BF16), preferred_element_type=F32)
        part[pi, pl.ds(off, TM), :] = r1
        x = pltpu.bitcast(lhs[li + z(), :, pl.ds(h, h)], BF16)
        r2 = jnp.dot(x, pltpu.bitcast(wp[wi, pl.ds(h // 2, h // 2), :], BF16), preferred_element_type=F32)
        r = part[pi + z(), pl.ds(off, TM), :] + r2
        return r, slabs(r1) + slabs(r2)

    def half_proj(sec, hf, c):
        dst, off = ((q_s, 0), (k0_s, HALO), (v_s, HALO))[sec]
        h = D // 2
        x = pltpu.bitcast(xu[z(), :, pl.ds(hf * h, h)], BF16)
        r = jnp.dot(x, pltpu.bitcast(wp[sec * 8 + c, pl.ds(hf * h // 2, h // 2), :], BF16),
                    preferred_element_type=F32)
        dst[c, pl.ds(off, TM), :] = dst[c + z(), pl.ds(off, TM), :] + r if hf else r
        return slabs(r)

    def b_proj(slot, sec, c):
        dst, off = ((q_s, 0), (k_s, HALO), (v_s, HALO))[sec]
        r, toks = mm2(xu, slot, sec * 8 + c, dst, c, off)
        dst[c, pl.ds(off, TM), :] = r
        return toks

    cexp = (DH ** -0.5) * math.log2(math.e)
    neg = -1e9 / (DH ** -0.5)
    flip = lane ^ 1

    def soft_units(t, rg):
        r0 = rg * 8
        st = {'ls': []}
        kb = k0_s if isinstance(t, int) and t == 0 else k_s

        def logits(ws):
            zi = z()
            q = [q_s[zi + c, pl.ds(r0, 8), :] for c in range(8)]
            for w in ws:
                acc = q[0] * kb[zi, pl.ds(HALO + r0 - DIL * w, 8), :]
                for c in range(1, 8):
                    acc = acc + q[c] * kb[zi + c, pl.ds(HALO + r0 - DIL * w, 8), :]
                acc = acc + pltpu.roll(acc, 64, 1)
                acc = acc + jnp.take_along_axis(acc, flip, axis=1)
                if r0 - DIL * w < 0 and not (isinstance(t, int) and t > 0):
                    acc = jnp.where(row + (t * TM + r0 - DIL * w) >= 0, acc, neg)
                st['ls'].append(acc)
            if len(st['ls']) == WIN:
                ls = st['ls']
                m = functools.reduce(jnp.maximum, ls)
                ps = [jnp.exp2((l - m) * cexp) for l in ls]
                inv_den = 1.0 / tsum(ps)
                for w in range(WIN):
                    p_s[w, pl.ds(r0, 8), :] = ps[w] * inv_den
        return [('soft', 68, P(logits, range(0, 4))), ('soft', 108, P(logits, range(4, 8)))]

    def av_units(c, dyn=True):
        def av(rbs):
            for rb in rbs:
                r0 = rb * 16
                zi = z()
                cv = zi + c if dyn else c
                acc = p_s[zi, pl.ds(r0, 16), :] * v_s[cv, pl.ds(HALO + r0, 16), :]
                for w in range(1, WIN):
                    acc = acc + p_s[zi + w, pl.ds(r0, 16), :] * v_s[cv, pl.ds(HALO + r0 - DIL * w, 16), :]
                o_s[c, pl.ds(r0, 16), :] = acc.astype(BF16)
            if rbs[-1] == TM // 16 - 1:
                ou[0, :, pl.ds(c * 128, 128)] = pltpu.bitcast(o_s[c + z()], U32)
        return [('av', 64, P(av, (rb, rb + 1))) for rb in range(0, TM // 16, 2)]

    def b_out(t, c):
        r, toks = mm2(ou, 0, 24 + c, acc_s, c % 2, 0)
        ob_v[t, :, pl.ds(c * 128, 128)] = r.astype(BF16)
        return toks

    def gate(kind, tok):
        if kind == 'conv':
            ug_s[6 * 16 * NB + zero] = tok
        elif kind == 'x':
            x_v[NSTEP + zero, pl.ds(0, 16), pl.ds(0, 128)] = pltpu.bitcast(tok, BF16)
        elif kind == 'soft':
            q_s[8 + zero, pl.ds(0, 8), :] = tok
        elif kind == 'av':
            p_s[8 + zero, pl.ds(0, 8), :] = tok
        elif kind == 'wv':
            w_v[32 + zero, pl.ds(0, 16), :] = pltpu.bitcast(tok, BF16)
        elif kind == 'wta':
            wt_a[8 + zero, pl.ds(0, 8), :] = pltpu.bitcast(tok, U32)
        elif kind == 'wtb':
            wt_b[8 + zero, pl.ds(0, 8), :] = pltpu.bitcast(tok, U32)
        elif kind == 'prep':
            kf_s[pl.ds(pl.multiple_of(S + 8 + zero * 8, 8), 8), :] = tok

    def a_consts(t):
        cs = pl.ds(al(t, CH), CH)
        skt_all = sk_ref[:, cs].astype(F32)
        sd = jnp.sum(jnp.where(row == t, sd_ref[...].astype(F32), 0.0), axis=0, keepdims=True)
        return [skt_all[d:d + 1, :] for d in range(KS)], sd

    def halo(ref, src=None):
        ref[:, pl.ds(0, HALO), :] = (ref if src is None else src)[:, pl.ds(TM, HALO), :]

    def pace(toks, units, lead=0):
        total = sum(u[1] for u in units)
        done = 0
        last = {}
        for kind, cost, fn in units:
            i = (len(toks) + lead) * done // total - lead
            if i >= 0 and last.get(kind) != i:
                gate(kind, toks[i])
                last[kind] = i
            fn()
            done += cost

    def merge(*lists):
        items = []
        for l in lists:
            if not l:
                continue
            tot = sum(u[1] for u in l)
            acc = 0
            for u in l:
                items.append((acc / tot, len(items), u))
                acc += u[1]
        return [u for _, _, u in sorted(items, key=lambda x: x[:2])]

    def emit(units):
        for u in units:
            u[2]()

    def tiny(i):
        return pltpu.make_async_copy(w_hbm.at[pl.ds(0, 16), pl.ds(0, 128)], tiny_v.at[i], sem_w.at[32 + i])

    nstart = [0]

    def start(ws, ins):
        for t, n in ins:
            in_copy(t, n).start()
        for sec in ws:
            for n in range(8):
                wo_copy(n).start()
        tiny(nstart[0]).wait()
        nstart[0] += 1

    def w_wait(sec):
        for n in range(8):
            wo_copy(n).wait()

    def in_wait(*tn):
        for t, n in tn:
            in_copy(t, n).wait()

    def soft_rows(t, a, b):
        return [u for rg in range(a, b) for u in soft_units(t, rg)]

    def prep_pair(t, c, skt):
        return prep_units(t, 2 * c, skt) + prep_units(t, 2 * c + 1, skt)

    def dft_pair(t, c, sd):
        toks = a_inv(t, 2 * c)
        a_inv(t, 2 * c + 1)
        toks += a_fwd(t + 1, 2 * c, sd)
        a_fwd(t + 1, 2 * c + 1, sd)
        return toks

    def tail_phases(t, extra, hook=None):
        halo(k_s, k0_s if extra else None)
        conv = [u for g in range(16) for u in conv_units(g)]
        ctot = sum(u[1] for u in conv)
        cdone = 0
        cw = CONV_W1 if extra else CONV_W
        for k in range(24):
            ph, c = divmod(k, 8)
            if hook is not None and k == 8:
                hook()
            toks = b_out(t, c) if ph == 2 else b_proj((t + 1) % 2, 1 - ph, c)
            if ph == 2:
                gate('x', toks[4])
                t2 = t + 2 if isinstance(t, int) else jnp.minimum(t + 2, NSTEP - 1)
                xu[t % 2, pl.ds(16 * c, 16), :] = pltpu.bitcast(x_v[t2, pl.ds(32 * c, 32), :], U32)
            mine = []
            while conv and cdone < ctot * sum(cw[:k + 1]) / sum(cw):
                cdone += conv[0][1]
                mine.append(conv.pop(0))
            units = merge(mine, av_units(c) if ph == 0 else [], extra.get(k, []))
            if units:
                pace(toks[:TAIL] if k == 23 else toks, units)
        copy_a(t).start()
        copy_b(t).start()

    for n in range(3):
        first_copy(0, n).start()
    small = [pltpu.make_async_copy(src, dst, sem_c.at[i]) for i, (src, dst) in enumerate(
        ((zero_hbm, zero_ref), (sk_hbm, sk_ref), (sd_hbm, sd_ref), (fwd_hbm, fwd_ref),
         (inv_hbm, inv_ref)))]
    for cp in small:
        cp.start()
    for i in range(NTINY):
        tiny(i).start()
    k0_s[:, pl.ds(0, HALO), :] = jnp.zeros((8, HALO, 128), F32)
    v_s[:, pl.ds(0, HALO), :] = jnp.zeros((8, HALO, 128), F32)
    kf_s[pl.ds(0, 8), :] = jnp.zeros((8, 128), F32)
    start([], [])
    for n in range(3):
        first_copy(1, n).start()
    for cp in small:
        cp.wait()
    zero = zero_ref[0]
    for n in range(3):
        first_copy(0, n).wait()
    for n in range(8):
        wh_copy(0, n).start()
    start([], [(0, 3)])
    skt, sd = a_consts(0)
    for c in range(8):
        if c == 4:
            for n in range(8):
                wh_copy(1, n).start()
            for n in range(3):
                first_copy(1, n).wait()
        if c % 4 == 0:
            emit(prep_pair(0, c, skt))
        toks = a_fwd(0, 2 * c, sd)
        a_fwd(0, 2 * c + 1, sd)
        if c % 4 < 3:
            pace(toks[:12], prep_pair(0, c + 1, skt), 4)
    conv = [u for g in range(16) for u in conv_units(g)]
    per = len(conv) // 16
    emit(conv[:PRO_G[0] * per])
    nxt_in = ((1, 3), (0, 4), (1, 0), (1, 1), (1, 2))

    def ready(p):
        if p + 2 < 6:
            for n in range(8):
                wh_copy(p + 2, n).start()
        elif p == 4:
            for tn in nxt_in:
                in_copy(*tn).start()
        for n in range(8):
            wh_copy(p, n).wait()
        if p == 0:
            in_wait((0, 3))
            stage_x(0, 0)
        sec, hf = (1, 0, 2)[p // 2], p % 2
        lanes = [lane_units(sec, c)[4 * hf:4 * hf + 4] for c in range(8)]
        return sel_units(sec)[32 * hf:32 * hf + 32], lanes

    soft = soft_rows(0, 0, 32)
    fills = [conv[PRO_G[p] * per:PRO_G[p + 1] * per] for p in range(4)]
    fills += [soft[:PRO_SOFT], soft[PRO_SOFT:]]
    sel, lanes = ready(0)
    emit(sel + lanes[0] + lanes[1])
    for p in range(6):
        fill = fills[p]
        slots = (0, 1, 2, 3, 6, 7) if p < 5 else (0, 1, 2, 3, 4, 5, 6)
        for c in range(8):
            if c == 4 and p < 5:
                sel, nxt = ready(p + 1)
            toks = half_proj((1, 0, 2)[p // 2], p % 2, c)
            units = [lanes[c + 2] if c < 6 else nxt[c - 6] if p < 5 else []]
            if c in slots:
                i = slots.index(c)
                units.append(fill[len(fill) * i // len(slots):len(fill) * (i + 1) // len(slots)])
            elif p < 5:
                units.append(sel[16 * (c - 4):16 * (c - 3)])
            units = merge(*units)
            if units:
                pace(toks[:12] if c == 3 else toks, units)
        lanes = nxt
    for n in range(8):
        wo_copy(n).start()
    in_copy(2, 3).start()
    in_wait(*nxt_in)
    stage_x(1, 1)
    skt, sd = a_consts(1)
    emit(prep_pair(1, 0, skt))
    for e in range(8):
        toks = dft_pair(0, e, sd)
        if e < 7:
            pace(toks[:20], prep_pair(1, e + 1, skt), 4)

    def hook():
        w_wait(3)
        in_wait((2, 3))
        start([], [(1, 4), (2, 0), (2, 1), (2, 2), (3, 3)])
    tail_phases(0, {8 + c: wo_units(c) for c in range(8)}, hook)

    assert nstart[0] == NTINY

    def loop(t, carry):
        in_copy(t + 1, 4).start()

        @pl.when(t + 3 < NSTEP)
        def _():
            in_copy(t + 3, 3).start()

        @pl.when(t + 2 < NSTEP)
        def _():
            for n in range(3):
                in_copy(t + 2, n).start()
            in_wait((t + 2, 3))

        in_wait((t, 4), (t + 1, 0), (t + 1, 1), (t + 1, 2))

        halo(v_s)
        skt, sd = a_consts(t + 1)
        for c in range(8):
            toks = b_proj(t % 2, 2, c)
            if c == 0:
                pace(toks[:16], prep_pair(t + 1, 0, skt), 2)
            toks = toks + dft_pair(t, c, sd)
            soft = soft_rows(1, 4 * c, 4 * c + 4)
            if c < 7:
                pace(toks, merge(soft, prep_pair(t + 1, c + 1, skt)), LEAD if c == 0 else 0)
            else:
                pace(toks[:FIN], soft)
        tail_phases(t, {})
        return carry
    jax.lax.fori_loop(1, NSTEP - 1, loop, 0)

    t = NSTEP - 1
    in_wait((t, 4))
    halo(v_s)
    for c in range(8):
        toks = b_proj(t % 2, 2, c)
        if c < 5:
            pace(toks, [u for rg in range(32) if rg * 5 // 32 == c for u in soft_units(t, rg)],
                 LEAD if c == 0 else 0)
        else:
            pace(toks, [u for cc in ((0, 1), (2, 3), (4, 5))[c - 5] for u in av_units(cc, False)])
    toks = []
    for i in range(NB):
        tk = a_inv(t, i)
        if i % 2 == 0:
            toks += tk
    pace(toks[:40], av_units(6, False) + av_units(7, False))
    copy_a(t).start()
    for c in range(8):
        b_out(t, c)
        if c % 2 == 1:
            copy_b_last(c // 2).start()
    for s in range(NSTEP - 1):
        copy_a(s).wait()
        copy_b(s).wait()
    copy_a(t).wait()
    for n in range(4):
        copy_b_last(n).wait()


@jax.jit
def pallas_concat_heads__ssm_conv_h3__sliding_local_dilated__prompt_kernel(
    A_q, A_k, A_v, A_shift_k, A_ssm_k, A_ssm_D, B_x, B_wqkv, B_wo,
):
    fwd, inv = _dft_consts()
    fwd = jnp.asarray(_pack_rows(fwd))
    inv = jnp.asarray(_pack_rows(inv))
    hbm = pl.BlockSpec(memory_space=pl.ANY)
    out = pl.pallas_call(
        _kernel,
        in_specs=[hbm] * 12,
        out_specs=hbm,
        out_shape=jax.ShapeDtypeStruct((S, 2 * D), BF16),
        scratch_shapes=[
            pltpu.VMEM((NSTEP, S, CH), BF16),
            pltpu.VMEM((NSTEP, S, CH), BF16),
            pltpu.VMEM((NSTEP, S, CH), BF16),
            pltpu.VMEM((NSTEP, CH, S), BF16),
            pltpu.VMEM((NSTEP + 1, TM, D), BF16),
            pltpu.VMEM((33, D, 128), BF16),
            pltpu.VMEM((32, D // 2, 128), U32),
            pltpu.VMEM((9, D // 2, 128), U32),
            pltpu.VMEM((9, D // 2, 128), U32),
            pltpu.VMEM((2, TM // 2, D), U32),
            pltpu.VMEM((1, TM // 2, D), U32),
            pltpu.VMEM((2, TM, 128), F32),
            pltpu.VMEM((9, TM, 128), F32),
            pltpu.VMEM((8, TM + HALO, 128), F32),
            pltpu.VMEM((8, TM + HALO, 128), F32),
            pltpu.VMEM((WIN + 1, TM, 128), F32),
            pltpu.VMEM((8, TM, 128), BF16),
            pltpu.VMEM((S + 16, 128), F32),
            pltpu.VMEM((S, 128), BF16),
            pltpu.VMEM((6 * 16 * NB + 1, 8, 128), F32),
            pltpu.VMEM((NB, 2 * BL, 128), BF16),
            pltpu.VMEM((NSTEP, S, CH), BF16),
            pltpu.VMEM((NSTEP, TM, D), BF16),
            pltpu.VMEM((NTINY, 16, 128), BF16),
            pltpu.VMEM((8, TM + HALO, 128), F32),
            pltpu.SemaphoreType.DMA((NSTEP, 5)),
            pltpu.SemaphoreType.DMA((32 + NTINY,)),
            pltpu.SemaphoreType.DMA((NSTEP, 5)),
            pltpu.SemaphoreType.DMA((NH, 3)),
            pltpu.SemaphoreType.DMA((6, 8)),
            pltpu.VMEM((KS, D), BF16),
            pltpu.VMEM((NSTEP, CH), BF16),
            pltpu.VMEM(fwd.shape, U32),
            pltpu.VMEM(inv.shape, U32),
            pltpu.SemaphoreType.DMA((5,)),
            pltpu.SMEM((NZ,), jnp.int32),
        ],
        compiler_params=pltpu.CompilerParams(vmem_limit_bytes=100 * 1024 * 1024),
    )(jnp.zeros((NZ,), jnp.int32), A_q.reshape(S, D), A_k.reshape(S, D), A_v.reshape(S, D),
      A_shift_k.T, A_ssm_k, A_ssm_D.reshape(NSTEP, CH),
      B_x.reshape(S, D), B_wqkv, B_wo, fwd, inv)
    return out.reshape(1, S, 2 * D)
```
